```python
import jax
import jax.numpy as jnp

def _softmax(x, axis=-1):
    return jax.nn.softmax(x, axis=axis)
def _gelu(x):
    return jax.nn.gelu(x, approximate=True)
def _silu(x):
    return jax.nn.silu(x)
def _sigmoid(x):
    return jax.nn.sigmoid(x)
def _layernorm(x, axis=-1, eps=1e-5):
    m = jnp.mean(x, axis=axis, keepdims=True)
    v = jnp.var(x, axis=axis, keepdims=True)
    return (x - m) / jnp.sqrt(v + eps)
def _scatter_add(tgt, idx, src, axis=0):
    return tgt.at[idx].add(src)
def _segment_sum(src, seg, n):
    return jax.ops.segment_sum(src, seg, n)
class _Rng:
    def __init__(self, key):
        self._k = key
    def _next(self):
        self._k, sub = jax.random.split(self._k)
        return sub
    def normal(self, shape):
        return jax.random.normal(self._next(), shape, dtype=jnp.bfloat16)
    def randint(self, lo, hi, shape):
        return jax.random.randint(self._next(), shape, lo, hi, dtype=jnp.int32)
    def uniform(self, shape, lo=0.0, hi=1.0):
        return jax.random.uniform(self._next(), shape, jnp.bfloat16, lo, hi)
    def permutation(self, n):
        return jax.random.permutation(self._next(), n)


kernel_name = 'interleave_layers__sliding_block_cached__moe_arch_mod__decode'

def setup_inputs():
    _rng = _Rng(jax.random.key(int.from_bytes(__import__("os").urandom(4), "little")))
    _w = (lambda a: (lambda t: t.astype(jnp.bfloat16) if jnp.issubdtype(t.dtype, jnp.floating) else t)(jnp.asarray(a)))
    def _A_setup():
        B, Sq, D = 4, 1, 640
        Hq, Hkv, Sk, Dh = 32, 32, 4096, 192
        assert Hq % Hkv == 0, (Hq, Hkv)
        return {
            "x": _w((lambda *s: _rng.normal(s) * 0.05)(B, Sq, D)),
            "k_cache": _w((lambda *s: _rng.normal(s) * 0.05)(B, Hkv, Sk, Dh)),
            "v_cache": _w((lambda *s: _rng.normal(s) * 0.05)(B, Hkv, Sk, Dh)),
            "wq": _w((lambda *s: _rng.normal(s) * 0.05)(D, Hq * Dh) * (D ** -0.5)),
            "wo": _w((lambda *s: _rng.normal(s) * 0.05)(Hq * Dh, D) * ((Hq * Dh) ** -0.5)),
        }
    _A_in = _A_setup()

    def _B_setup():
        B, S, D, F, C = 4, 1, 640, 1536, 1
        return {
            "x": _w((lambda *s: _rng.normal(s) * 0.05)(B, S, D)),
            "w_r": _w((lambda *s: _rng.normal(s) * 0.05)(D)),
            "w_gate": _w((lambda *s: _rng.normal(s) * 0.05)(D, F)),
            "w_up": _w((lambda *s: _rng.normal(s) * 0.05)(D, F)),
            "w_down": _w((lambda *s: _rng.normal(s) * 0.05)(F, D)),
        }
    _B_in = _B_setup()

    return {
        "A_x": _A_in["x"],
        "A_k_cache": _A_in["k_cache"],
        "A_v_cache": _A_in["v_cache"],
        "A_wq": _A_in["wq"],
        "A_wo": _A_in["wo"],
        "B_x": _B_in["x"],
        "B_w_r": _B_in["w_r"],
        "B_w_gate": _B_in["w_gate"],
        "B_w_up": _B_in["w_up"],
        "B_w_down": _B_in["w_down"],
    }

def reference(A_x, A_k_cache, A_v_cache, A_wq, A_wo, B_x, B_w_r, B_w_gate, B_w_up, B_w_down):
    def _A_ref(x, k_cache, v_cache, wq, wo):
        B, Sq, D = x.shape
        Hq, Dh = 32, 192
        Hkv, Sk = k_cache.shape[1], k_cache.shape[2]
        W = min(4096, max(256, Sk // 4))
        rep = Hq // Hkv
        q = (lambda x, *d: x.transpose(*d))((x @ wq).reshape(B, Sq, Hq, Dh), 0, 2, 1, 3)
        k = jnp.repeat(k_cache[:, :, Sk - W:, :], rep, axis=1)
        v = jnp.repeat(v_cache[:, :, Sk - W:, :], rep, axis=1)
        scores = jnp.einsum("bhqd,bhkd->bhqk", q, k) * (Dh ** -0.5)
        p = _softmax(scores, axis=-1)
        o = jnp.einsum("bhqk,bhkd->bhqd", p, v)
        return (lambda x, *d: x.transpose(*d))(o, 0, 2, 1, 3).reshape(B, Sq, Hq * Dh) @ wo

    def _B_ref(x, w_r, w_gate, w_up, w_down):
        B, S, D = x.shape
        C = 1
        r = x @ w_r
        idx = jnp.argsort(-r, axis=-1)[:, :C]
        idx_e = jnp.repeat(idx.reshape(B, C, 1), D, axis=2)
        x_sel = jnp.take_along_axis(x, idx_e, axis=1)
        g = _silu(x_sel @ w_gate)
        u = x_sel @ w_up
        y = (g * u) @ w_down
        r_sel = _sigmoid(jnp.take_along_axis(r, idx, axis=1))
        y = y * r_sel.reshape(B, C, 1)
        b_off = (jnp.arange(B) * S).reshape(B, 1)
        flat_idx = (idx + b_off).reshape(B * C)
        zero = (x * 0.0).reshape(B * S, D)
        upd = _scatter_add(zero, flat_idx, y.reshape(B * C, D), axis=0)
        return x + upd.reshape(B, S, D)

    x = A_x
    x = x + _A_ref(_layernorm(x, axis=-1), A_k_cache, A_v_cache, A_wq, A_wo)
    x = x + _B_ref(_layernorm(x, axis=-1), B_w_r, B_w_gate, B_w_up, B_w_down)
    x = x + _A_ref(_layernorm(x, axis=-1), A_k_cache, A_v_cache, A_wq, A_wo)
    x = x + _B_ref(_layernorm(x, axis=-1), B_w_r, B_w_gate, B_w_up, B_w_down)
    return x
```

```python
import functools

import jax
import jax.numpy as jnp
import numpy as np
from jax import lax
import jax.experimental.pallas as pl
import jax.experimental.pallas.tpu as pltpu

_D = 640
_H = 32
_DH = 192
_SK = 4096
_W = 1024
_F = 1536
_B = 4
_G = 8
_NG = _H // _G
_GD = _G * _DH
_NJ = _W // 128
_EPS = 1e-5

_BF = jnp.bfloat16
_F32 = jnp.float32
_U32 = jnp.uint32


def _mm(a, b):
    return jnp.dot(a, b, preferred_element_type=_F32)


def _mm_nt(a, b):
    return lax.dot_general(a, b, (((1,), (1,)), ((), ())), preferred_element_type=_F32)


def _layernorm(x):
    m = jnp.mean(x, axis=-1, keepdims=True)
    xc = x - m
    v = jnp.mean(xc * xc, axis=-1, keepdims=True)
    return xc / jnp.sqrt(v + _EPS)


def _kernel(x_ref, wr_ref, k_hbm, v_hbm, wq_hbm, wo_hbm, wg_hbm, wu_hbm, wd_hbm,
            o_ref,
            kbuf, vbuf, wq_s, wo_s, wg_s, wu_s, wd_s, xs, os_,
            ksem, vsem, wsem):
    kd = kbuf.bitcast(_BF)
    vd = vbuf.bitcast(_BF)
    wq_d = wq_s.bitcast(_BF)
    wo_d = wo_s.bitcast(_BF)
    wg_d = wg_s.bitcast(_BF)
    wu_d = wu_s.bitcast(_BF)
    wd_d = wd_s.bitcast(_BF)

    def w_copies(src, dst, sem_i):
        n = dst.shape[0]
        return [pltpu.make_async_copy(src.at[:, pl.ds(128 * j, 128)], dst.at[j], wsem.at[sem_i])
                for j in range(n)]

    def k_copy(b, j):
        slot = b % 2
        return pltpu.make_async_copy(
            k_hbm.at[b, :, :, pl.ds(_SK - _W + 128 * j, 128)], kd.at[slot, j], ksem.at[slot])

    def v_copy(b, g, j):
        slot = b % 2
        return pltpu.make_async_copy(
            v_hbm.at[b, pl.ds(g * _G, _G), :, pl.ds(_SK - _W + 128 * j, 128)],
            vd.at[slot, j, pl.ds(g * _G, _G)], vsem.at[slot, g])

    wq_c = w_copies(wq_hbm, wq_d, 0)
    wo_c = w_copies(wo_hbm, wo_d, 1)
    wg_c = w_copies(wg_hbm, wg_d, 2)
    wu_c = w_copies(wu_hbm, wu_d, 3)
    wd_c = w_copies(wd_hbm, wd_d, 4)

    for c in wq_c + wo_c + wg_c + wu_c + wd_c:
        c.start()
    for j in range(_NJ):
        k_copy(0, j).start()
    for g in range(_NG):
        for j in range(_NJ):
            v_copy(0, g, j).start()

    xs[...] = jnp.zeros(xs.shape, _F32)
    xs[0:_B, :] = x_ref[...].astype(_F32)
    wr = wr_ref[...].astype(_F32).reshape(1, _D)

    row = lax.broadcasted_iota(jnp.int32, (_G, _GD), 0)
    col = lax.broadcasted_iota(jnp.int32, (_G, _GD), 1)
    bd_mask = (col >= row * _DH) & (col < (row + 1) * _DH)

    for c in wq_c + wo_c + wg_c + wu_c + wd_c:
        c.wait()

    def ld(ref_slice):
        return pltpu.bitcast(ref_slice, _BF)

    def batch_body(b, carry):
        slot = b % 2
        x0 = jnp.broadcast_to(xs[pl.ds(b, 1), :], (8, _D))

        def layer_body(l, x):
            xn = _layernorm(x).astype(_BF)

            @pl.when(l == 0)
            def _():
                for j in range(_NJ):
                    k_copy(b, j).wait()

                @pl.when(b + 1 < _B)
                def _():
                    for j in range(_NJ):
                        k_copy(b + 1, j).start()

            def group_body(g, acc):
                nq = _GD // 128
                q = jnp.concatenate(
                    [_mm(xn, ld(wq_s[g * nq + jj])) for jj in range(nq)], axis=1)
                qbd = jnp.where(bd_mask, q.astype(_BF).astype(_F32), 0.0).astype(_BF)
                s = jnp.concatenate(
                    [_mm(qbd, ld(kbuf[slot, j, pl.ds(g * _G, _G)]).reshape(_GD, 128))
                     for j in range(_NJ)], axis=1)
                s = s * (_DH ** -0.5)
                m = jnp.max(s, axis=-1, keepdims=True)
                p = jnp.exp(s - m)
                lsum = jnp.sum(p, axis=-1, keepdims=True)
                pb = p.astype(_BF)

                @pl.when(l == 0)
                def _():
                    for j in range(_NJ):
                        v_copy(b, g, j).wait()

                    @pl.when(b + 1 < _B)
                    def _():
                        for j in range(_NJ):
                            v_copy(b + 1, g, j).start()

                o = None
                for j in range(_NJ):
                    t = _mm_nt(pb[:, 128 * j:128 * (j + 1)],
                               ld(vbuf[slot, j, pl.ds(g * _G, _G)]).reshape(_GD, 128))
                    o = t if o is None else o + t
                o = jnp.where(bd_mask, o / lsum, 0.0).astype(_BF)
                upd = jnp.concatenate(
                    [_mm(o, ld(wo_s[jn, pl.ds(g * (_GD // 2), _GD // 2), :]))
                     for jn in range(_D // 128)], axis=1)
                return acc + upd

            acc = lax.fori_loop(0, _NG, group_body, jnp.zeros((8, _D), _F32))
            attn = jnp.sum(acc, axis=0, keepdims=True)
            x = x + attn

            xn32 = _layernorm(x)
            xn = xn32.astype(_BF)
            xnr = xn.astype(_F32)
            r = jnp.sum(xnr * wr, axis=-1, keepdims=True)
            nf = _F // 128
            gate = jnp.concatenate([_mm(xn, ld(wg_s[jj])) for jj in range(nf)], axis=1)
            up = jnp.concatenate([_mm(xn, ld(wu_s[jj])) for jj in range(nf)], axis=1)
            h = (gate * jax.nn.sigmoid(gate) * up).astype(_BF)
            y = jnp.concatenate([_mm(h, ld(wd_s[jn])) for jn in range(_D // 128)], axis=1)
            x = x + (xnr + y * jax.nn.sigmoid(r))
            return x

        x = lax.fori_loop(0, 2, layer_body, x0)
        os_[pl.ds(b, 1), :] = x[0:1, :]
        return carry

    os_[...] = jnp.zeros(os_.shape, _F32)
    lax.fori_loop(0, _B, batch_body, 0)
    o_ref[...] = os_[0:_B, :].astype(o_ref.dtype)


@jax.jit
def pallas_interleave_layers__sliding_block_cached__moe_arch_mod__decode_kernel(
    A_x: jax.Array,
    A_k_cache: jax.Array,
    A_v_cache: jax.Array,
    A_wq: jax.Array,
    A_wo: jax.Array,
    B_x: jax.Array,
    B_w_r: jax.Array,
    B_w_gate: jax.Array,
    B_w_up: jax.Array,
    B_w_down: jax.Array,
):
    del B_x
    kt = jnp.transpose(A_k_cache, (0, 1, 3, 2))
    vt = jnp.transpose(A_v_cache, (0, 1, 3, 2))
    x2 = A_x.reshape(_B, _D)

    any_spec = pl.BlockSpec(memory_space=pl.ANY)
    vmem_spec = pl.BlockSpec(memory_space=pltpu.VMEM)
    out = pl.pallas_call(
        _kernel,
        out_shape=jax.ShapeDtypeStruct((_B, _D), A_x.dtype),
        in_specs=[vmem_spec, vmem_spec] + [any_spec] * 7,
        out_specs=vmem_spec,
        scratch_shapes=[
            pltpu.VMEM((2, _NJ, _H, _DH // 2, 128), _U32),
            pltpu.VMEM((2, _NJ, _H, _DH // 2, 128), _U32),
            pltpu.VMEM((_H * _DH // 128, _D // 2, 128), _U32),
            pltpu.VMEM((_D // 128, _H * _DH // 2, 128), _U32),
            pltpu.VMEM((_F // 128, _D // 2, 128), _U32),
            pltpu.VMEM((_F // 128, _D // 2, 128), _U32),
            pltpu.VMEM((_D // 128, _F // 2, 128), _U32),
            pltpu.VMEM((8, _D), _F32),
            pltpu.VMEM((8, _D), _F32),
            pltpu.SemaphoreType.DMA((2,)),
            pltpu.SemaphoreType.DMA((2, _NG)),
            pltpu.SemaphoreType.DMA((5,)),
        ],
        compiler_params=pltpu.CompilerParams(vmem_limit_bytes=100 * 1024 * 1024),
    )(x2, B_w_r, kt, vt, A_wq, A_wo, B_w_gate, B_w_up, B_w_down)
    return out.reshape(_B, 1, _D)
```

```python
import functools
import contextlib
import jax
import jax.numpy as jnp
import numpy as np
from jax import lax
import jax.experimental.pallas as pl
import jax.experimental.pallas.tpu as pltpu

_D = 640; _H = 32; _DH = 192; _SK = 4096; _W = 1024; _F = 1536; _B = 4; _NJ = 8
_EPS = 1e-5
_BF = jnp.bfloat16; _F32 = jnp.float32; _U32 = jnp.uint32

V_CHUNKS = [(0, 8), (8, 8), (16, 8), (24, 4), (28, 2), (30, 2)]
GROUPS_L1 = [(4*g, 4, 'V') for g in range(7)] + [(28, 4, 'M')]
PROFILE = False

def scope(name):
    return jax.named_scope(name) if PROFILE else contextlib.nullcontext()

def mm(a, b): return jnp.dot(a, b, preferred_element_type=_F32)
def mm_nt(a, b): return lax.dot_general(a, b, (((1,), (1,)), ((), ())), preferred_element_type=_F32)
def ld(r): return pltpu.bitcast(r, _BF)

def layernorm(x):
    m = jnp.mean(x, axis=-1, keepdims=True)
    xc = x - m
    v = jnp.mean(xc * xc, axis=-1, keepdims=True)
    return xc / jnp.sqrt(v + _EPS)

def bd_mask(gs):
    gd = gs * _DH
    row = lax.broadcasted_iota(jnp.int32, (8, gd), 0)
    col = lax.broadcasted_iota(jnp.int32, (8, gd), 1)
    return (col >= row * _DH) & (col < (row + 1) * _DH)

def probs(xn, kb, wq_s, h0, gs):
    gd = gs * _DH
    j0 = h0 * _DH // 128
    q = jnp.concatenate([mm(xn, ld(wq_s[j0 + jj])) for jj in range(gd // 128)], axis=1)
    qbd = jnp.where(bd_mask(gs), q, 0.0).astype(_BF)
    s = jnp.concatenate([mm(qbd, ld(kb[j, h0:h0 + gs]).reshape(gd, 128)) for j in range(_NJ)], axis=1)
    s = s * (_DH ** -0.5)
    m = jnp.max(s, axis=-1, keepdims=True)
    p = jnp.exp(s - m)
    return p / jnp.sum(p, axis=-1, keepdims=True)

def head_vpu(prow, vb, wo_s, h, yacc):
    a = None
    for j in range(_NJ):
        v = ld(vb[j, h]).astype(_F32)
        t = v * prow[:, 128 * j:128 * (j + 1)]
        a = t if a is None else a + t
    o = jnp.sum(a, axis=-1, keepdims=True)
    out = []
    for n in range(_D // 128):
        w = ld(wo_s[pl.ds(pl.multiple_of(h * (_DH // 2), 8), _DH // 2), 128 * n:128 * (n + 1)]).astype(_F32)
        c = (w * o).reshape(_DH // 8, 8, 128).sum(axis=0)
        out.append(c if yacc is None else yacc[n] + c)
    return out

def group_mxu(p, vb, wo_s, h0, gs):
    gd = gs * _DH
    pb = p.astype(_BF)
    o = None
    for j in range(_NJ):
        t = mm_nt(pb[:, 128 * j:128 * (j + 1)], ld(vb[j, h0:h0 + gs]).reshape(gd, 128))
        o = t if o is None else o + t
    o = jnp.where(bd_mask(gs), o, 0.0).astype(_BF)
    return jnp.concatenate([mm(o, ld(wo_s[h0 * 96:(h0 + gs) * 96, 128 * n:128 * (n + 1)])) for n in range(_D // 128)], axis=1)

def ffn(x, wr, wg_s, wu_s, wd_s):
    xn = layernorm(x).astype(_BF)
    xnr = xn.astype(_F32)
    r = jnp.sum(xnr * wr, axis=-1, keepdims=True)
    gate = jnp.concatenate([mm(xn, ld(wg_s[jj])) for jj in range(_F // 128)], axis=1)
    up = jnp.concatenate([mm(xn, ld(wu_s[jj])) for jj in range(_F // 128)], axis=1)
    h = (gate * jax.nn.sigmoid(gate) * up).astype(_BF)
    y = jnp.concatenate([mm(h, ld(wd_s[:, 128 * n:128 * (n + 1)])) for n in range(_D // 128)], axis=1)
    return x + (xnr + y * jax.nn.sigmoid(r))

def kernel(x_ref, wr_ref, k_hbm, v_hbm, wq_hbm, wo_hbm, wg_hbm, wu_hbm, wd_hbm, o_ref,
           kbuf, vbuf, wq_s, wo_s, wg_s, wu_s, wd_s, xs, os_, ps, ksem, vsem, wsem):
    kd = kbuf.bitcast(_BF); vd = vbuf.bitcast(_BF)

    def w_copies(src, dst, sem_i):
        d = dst.bitcast(_BF)
        return [pltpu.make_async_copy(src.at[:, pl.ds(128 * j, 128)], d.at[j], wsem.at[sem_i]) for j in range(d.shape[0])]
    def k_copy(b, j):
        return pltpu.make_async_copy(k_hbm.at[b, :, :, pl.ds(pl.multiple_of(_SK - _W + 128 * j, 128), 128)], kd.at[b % 2, j], ksem.at[b % 2])
    def v_copy(b, c, j):
        h0, n = V_CHUNKS[c]
        return pltpu.make_async_copy(v_hbm.at[b, pl.ds(h0, n), :, pl.ds(pl.multiple_of(_SK - _W + 128 * j, 128), 128)],
                                     vd.at[b % 2, j, pl.ds(h0, n)], vsem.at[b % 2, c])
    wo_c = pltpu.make_async_copy(wo_hbm, wo_s.bitcast(_BF), wsem.at[1])
    wd_c = pltpu.make_async_copy(wd_hbm, wd_s.bitcast(_BF), wsem.at[4])
    wcs = [w_copies(wq_hbm, wq_s, 0), [wo_c], w_copies(wg_hbm, wg_s, 2),
           w_copies(wu_hbm, wu_s, 3), [wd_c]]
    def ordered_starts(n, mk):
        def body(j, c):
            mk(j).start()
            return c
        lax.fori_loop(0, n, body, 0)
    def w_copy(src, dst, sem_i, j):
        return pltpu.make_async_copy(src.at[:, pl.ds(pl.multiple_of(128 * j, 128), 128)], dst.bitcast(_BF).at[j], wsem.at[sem_i])
    with scope("issue0"):
        ordered_starts(wq_s.shape[0], functools.partial(w_copy, wq_hbm, wq_s, 0))
        wo_c.start()
        ordered_starts(wg_s.shape[0], functools.partial(w_copy, wg_hbm, wg_s, 2))
        ordered_starts(wu_s.shape[0], functools.partial(w_copy, wu_hbm, wu_s, 3))
        wd_c.start()
        ordered_starts(_NJ, lambda j: k_copy(0, j))
        for c in range(len(V_CHUNKS)):
            ordered_starts(_NJ, lambda j, c=c: v_copy(0, c, j))

    xs[...] = jnp.zeros(xs.shape, _F32)
    xs[0:_B, :] = x_ref[...].astype(_F32)
    os_[...] = jnp.zeros(os_.shape, _F32)
    wr = wr_ref[...].astype(_F32).reshape(1, _D)
    with scope("waitw"):
        for cs in wcs:
            for c in cs: c.wait()

    def batch_body(b, carry):
        slot = b % 2
        kb = kbuf.at[slot]; vb = vbuf.at[slot]
        x = jnp.broadcast_to(xs[pl.ds(b, 1), :], (8, _D))
        xn = layernorm(x).astype(_BF)
        with scope("waitk"):
            for j in range(_NJ): k_copy(b, j).wait()
            @pl.when(b + 1 < _B)
            def _():
                for j in range(_NJ): k_copy(b + 1, j).start()
        with scope("scores1"):
            for g in range(4):
                ps[8 * g:8 * g + 8, :] = probs(xn, kb, wq_s, 8 * g, 8)
        yacc = tuple(jnp.zeros((8, 128), _F32) for _ in range(_D // 128))
        for c, (h0, n) in enumerate(V_CHUNKS):
            with scope(f"waitv{c}"):
                for j in range(_NJ): v_copy(b, c, j).wait()
                @pl.when(b + 1 < _B)
                def _():
                    for j in range(_NJ): v_copy(b + 1, c, j).start()
            with scope(f"pv1_{c}"):
                def pair(i, ya, h0=h0):
                    h = h0 + 2 * i
                    ya = head_vpu(ps[pl.ds(h, 1), :], vb, wo_s, h, ya)
                    ya = head_vpu(ps[pl.ds(h + 1, 1), :], vb, wo_s, h + 1, ya)
                    return tuple(ya)
                if n == 2:
                    yacc = pair(0, yacc)
                else:
                    yacc = lax.fori_loop(0, n // 2, pair, yacc)
        with scope("ffn1"):
            attn = jnp.concatenate([jnp.sum(y, axis=0, keepdims=True) for y in yacc], axis=1)
            x = x + attn
            x = ffn(x, wr, wg_s, wu_s, wd_s)
        with scope("attn2"):
            xn = layernorm(x).astype(_BF)
            yacc = None; macc = None
            for (h0, gs, path) in GROUPS_L1:
                p = probs(xn, kb, wq_s, h0, gs)
                if path == 'M':
                    u = group_mxu(p, vb, wo_s, h0, gs)
                    macc = u if macc is None else macc + u
                else:
                    for i in range(gs):
                        yacc = head_vpu(p[i:i + 1, :], vb, wo_s, h0 + i, yacc)
            attn = jnp.concatenate([jnp.sum(y, axis=0, keepdims=True) for y in yacc], axis=1)
            if macc is not None:
                attn = attn + jnp.sum(macc, axis=0, keepdims=True)
            x = x + attn
        with scope("ffn2"):
            x = ffn(x, wr, wg_s, wu_s, wd_s)
            os_[pl.ds(b, 1), :] = x[0:1, :]
        return carry

    lax.fori_loop(0, _B, batch_body, 0)
    o_ref[...] = os_[0:_B, :].astype(o_ref.dtype)


@jax.jit
def pallas_interleave_layers__sliding_block_cached__moe_arch_mod__decode_kernel(
    A_x, A_k_cache, A_v_cache, A_wq, A_wo, B_x, B_w_r, B_w_gate, B_w_up, B_w_down):
    del B_x
    kt = jnp.transpose(A_k_cache, (0, 1, 3, 2))
    vt = jnp.transpose(A_v_cache, (0, 1, 3, 2))
    x2 = A_x.reshape(_B, _D)
    any_spec = pl.BlockSpec(memory_space=pl.ANY)
    vmem_spec = pl.BlockSpec(memory_space=pltpu.VMEM)
    out = pl.pallas_call(
        kernel,
        out_shape=jax.ShapeDtypeStruct((_B, _D), A_x.dtype),
        in_specs=[vmem_spec, vmem_spec] + [any_spec] * 7,
        out_specs=vmem_spec,
        scratch_shapes=[
            pltpu.VMEM((2, _NJ, _H, _DH // 2, 128), _U32),
            pltpu.VMEM((2, _NJ, _H, _DH // 2, 128), _U32),
            pltpu.VMEM((_H * _DH // 128, _D // 2, 128), _U32),
            pltpu.VMEM((_H * _DH // 2, _D), _U32),
            pltpu.VMEM((_F // 128, _D // 2, 128), _U32),
            pltpu.VMEM((_F // 128, _D // 2, 128), _U32),
            pltpu.VMEM((_F // 2, _D), _U32),
            pltpu.VMEM((8, _D), _F32),
            pltpu.VMEM((8, _D), _F32),
            pltpu.VMEM((_H, _W), _F32),
            pltpu.SemaphoreType.DMA((2,)),
            pltpu.SemaphoreType.DMA((2, len(V_CHUNKS))),
            pltpu.SemaphoreType.DMA((5,)),
        ],
        compiler_params=pltpu.CompilerParams(vmem_limit_bytes=100 * 1024 * 1024),
    )(x2, B_w_r, kt, vt, A_wq, A_wo, B_w_gate, B_w_up, B_w_down)
    return out.reshape(_B, 1, _D)
```

```python
import functools
import contextlib
import jax
import jax.numpy as jnp
import numpy as np
from jax import lax
import jax.experimental.pallas as pl
import jax.experimental.pallas.tpu as pltpu

_D = 640; _H = 32; _DH = 192; _SK = 4096; _W = 1024; _F = 1536; _B = 4; _NJ = 8
_EPS = 1e-5
_BF = jnp.bfloat16; _F32 = jnp.float32; _U32 = jnp.uint32

V_CHUNKS = [(0, 8), (8, 8), (16, 8), (24, 4), (28, 2), (30, 2)]
GSIZES = (2,) * 16
PROFILE = False

def scope(name):
    return jax.named_scope(name) if PROFILE else contextlib.nullcontext()

def mm(a, b): return jnp.dot(a, b, preferred_element_type=_F32)
def ld(r): return pltpu.bitcast(r, _BF)

def layernorm(x):
    m = jnp.mean(x, axis=-1, keepdims=True)
    xc = x - m
    v = jnp.mean(xc * xc, axis=-1, keepdims=True)
    return xc / jnp.sqrt(v + _EPS)

def bd_mask(gs):
    gd = gs * _DH
    row = lax.broadcasted_iota(jnp.int32, (8, gd), 0)
    col = lax.broadcasted_iota(jnp.int32, (8, gd), 1)
    return (col >= row * _DH) & (col < (row + 1) * _DH)

def softmax_rows(s):
    s = s * (_DH ** -0.5)
    m = jnp.max(s, axis=-1, keepdims=True)
    p = jnp.exp(s - m)
    return p / jnp.sum(p, axis=-1, keepdims=True)

def probs(xn, kb, wq_s, h0, gs):
    gd = gs * _DH
    j0 = h0 * _DH // 128
    q = jnp.concatenate([mm(xn, ld(wq_s[j0 + jj])) for jj in range(gd // 128)], axis=1)
    qbd = jnp.where(bd_mask(gs), q, 0.0).astype(_BF)
    s = jnp.concatenate([mm(qbd, ld(kb[j, h0 * 96:(h0 + gs) * 96, :])) for j in range(_NJ)], axis=1)
    return softmax_rows(s)

def out_proj(o, wof, r0, yacc):
    out = []
    for n in range(_D // 128):
        w = wof[pl.ds(r0, _DH), 128 * n:128 * (n + 1)]
        c = (w * o).reshape(_DH // 8, 8, 128).sum(axis=0)
        out.append(c if yacc is None else yacc[n] + c)
    return out

def attn2(x, kb, vf, wq_s, wof):
    xn = layernorm(x).astype(_BF)
    ng = len(GSIZES)
    h0s = [sum(GSIZES[:i]) for i in range(ng)]
    qb = {}
    def do_q(gi):
        gs, h0 = GSIZES[gi], h0s[gi]
        nc = gs * _DH // 128; j0 = h0 * _DH // 128
        m = bd_mask(gs)
        qb[gi] = [jnp.where(m[:, 128 * c:128 * (c + 1)], mm(xn, ld(wq_s[j0 + c])), 0.0).astype(_BF) for c in range(nc)]
    yacc = None
    do_q(0)
    for gi in range(ng):
        gs, h0 = GSIZES[gi], h0s[gi]
        if gi + 1 < ng: do_q(gi + 1)
        qbd = jnp.concatenate(qb[gi], axis=1)
        s = jnp.concatenate([mm(qbd, ld(kb[j, h0 * 96:(h0 + gs) * 96, :])) for j in range(_NJ)], axis=1)
        p = softmax_rows(s)
        for i in range(gs):
            h = h0 + i
            a = None
            for j in range(_NJ):
                t = vf[j, h * _DH:(h + 1) * _DH, :] * p[i:i + 1, 128 * j:128 * (j + 1)]
                a = t if a is None else a + t
            o = jnp.sum(a, axis=-1, keepdims=True)
            yacc = out_proj(o, wof, h * _DH, yacc)
    attn = jnp.concatenate([jnp.sum(y, axis=0, keepdims=True) for y in yacc], axis=1)
    return x + attn

def ffn(x, wr, wg_s, wu_s, wd_s):
    xn = layernorm(x).astype(_BF)
    xnr = xn.astype(_F32)
    r = jnp.sum(xnr * wr, axis=-1, keepdims=True)
    gate = jnp.concatenate([mm(xn, ld(wg_s[jj])) for jj in range(_F // 128)], axis=1)
    up = jnp.concatenate([mm(xn, ld(wu_s[jj])) for jj in range(_F // 128)], axis=1)
    h = (gate * jax.nn.sigmoid(gate) * up).astype(_BF)
    y = jnp.concatenate([mm(h, ld(wd_s[:, 128 * n:128 * (n + 1)])) for n in range(_D // 128)], axis=1)
    return x + (xnr + y * jax.nn.sigmoid(r))

def kernel(x_hbm, wr_hbm, k_hbm, v_hbm, wq_hbm, wo_hbm, wg_hbm, wu_hbm, wd_hbm, o_ref,
           kbuf, vbuf, wq_s, wo_s, wg_s, wu_s, wd_s, vf, wof, x_s, wr_s, xs, os_, ps, ksem, vsem, wsem):
    def k_copy(b, j):
        return pltpu.make_async_copy(k_hbm.at[b, :, pl.ds(pl.multiple_of(_SK - _W + 128 * j, 128), 128)],
                                     kbuf.bitcast(_BF).at[b % 2, j], ksem.at[b % 2])
    def v_copy(b, c, j):
        h0, n = V_CHUNKS[c]
        return pltpu.make_async_copy(v_hbm.at[b, pl.ds(h0 * _DH, n * _DH), pl.ds(pl.multiple_of(_SK - _W + 128 * j, 128), 128)],
                                     vbuf.bitcast(_BF).at[b % 2, j, pl.ds(h0 * _DH, n * _DH)], vsem.at[b % 2, c])
    def w_copy(src, dst, sem_i, j):
        return pltpu.make_async_copy(src.at[:, pl.ds(pl.multiple_of(128 * j, 128), 128)], dst.bitcast(_BF).at[j], wsem.at[sem_i])
    wo_c = pltpu.make_async_copy(wo_hbm, wo_s.bitcast(_BF), wsem.at[1])
    wd_c = pltpu.make_async_copy(wd_hbm, wd_s.bitcast(_BF), wsem.at[4])
    x_c = pltpu.make_async_copy(x_hbm, x_s, wsem.at[5])
    wr_c = pltpu.make_async_copy(wr_hbm, wr_s, wsem.at[6])

    def ordered_starts(n, mk):
        def body(j, c):
            mk(j).start()
            return c
        lax.fori_loop(0, n, body, 0)
    def wait_all(n, mk):
        for j in range(n): mk(j).wait()

    with scope("issue0"):
        ordered_starts(wq_s.shape[0], functools.partial(w_copy, wq_hbm, wq_s, 0))
        x_c.start(); wr_c.start()
        wo_c.start()
        ordered_starts(wg_s.shape[0], functools.partial(w_copy, wg_hbm, wg_s, 2))
        ordered_starts(wu_s.shape[0], functools.partial(w_copy, wu_hbm, wu_s, 3))
        wd_c.start()
        ordered_starts(_NJ, lambda j: k_copy(0, j))
        for c in range(len(V_CHUNKS)):
            ordered_starts(_NJ, lambda j, c=c: v_copy(0, c, j))

    with scope("waitw"):
        x_c.wait(); wr_c.wait()
        xs[...] = jnp.zeros(xs.shape, _F32)
        xs[0:_B, :] = x_s[...].astype(_F32)
        os_[...] = jnp.zeros(os_.shape, _F32)
        wr = wr_s[...].astype(_F32).reshape(1, _D)
        wo_c.wait()
    with scope("mkwof"):
        def unpack_wo(h, c):
            wof[pl.ds(pl.multiple_of(h * _DH, 8), _DH), :] = ld(wo_s[pl.ds(pl.multiple_of(h * 96, 8), 96), :]).astype(_F32)
            return c
        lax.fori_loop(0, _H, unpack_wo, 0)
    with scope("waitw2"):
        wait_all(wq_s.shape[0], functools.partial(w_copy, wq_hbm, wq_s, 0))
        wait_all(wg_s.shape[0], functools.partial(w_copy, wg_hbm, wg_s, 2))
        wait_all(wu_s.shape[0], functools.partial(w_copy, wu_hbm, wu_s, 3))
        wd_c.wait()

    def batch_body(b, carry):
        slot = b % 2
        kb = kbuf.at[slot]; vb = vbuf.at[slot]
        x = jnp.broadcast_to(xs[pl.ds(b, 1), :], (8, _D))
        xn = layernorm(x).astype(_BF)
        with scope("waitk"):
            @pl.when(b + 1 < _B)
            def _():
                ordered_starts(_NJ, lambda j: k_copy(b + 1, j))
            wait_all(_NJ, lambda j: k_copy(b, j))
        with scope("scores1"):
            for g in range(4):
                ps[8 * g:8 * g + 8, :] = probs(xn, kb, wq_s, 8 * g, 8)
        yacc = tuple(jnp.zeros((8, 128), _F32) for _ in range(_D // 128))
        for c, (h0, n) in enumerate(V_CHUNKS):
            with scope(f"waitv{c}"):
                wait_all(_NJ, lambda j, c=c: v_copy(b, c, j))
                @pl.when(b + 1 < _B)
                def _():
                    ordered_starts(_NJ, lambda j, c=c: v_copy(b + 1, c, j))
            with scope(f"pv1_{c}"):
                def head1(h, ya):
                    prow = ps[pl.ds(h, 1), :]
                    a = None
                    r0 = pl.multiple_of(h * _DH, 8)
                    for j in range(_NJ):
                        v = ld(vb[j, pl.ds(pl.multiple_of(h * 96, 8), 96), :]).astype(_F32)
                        vf[j, pl.ds(r0, _DH), :] = v
                        t = v * prow[:, 128 * j:128 * (j + 1)]
                        a = t if a is None else a + t
                    o = jnp.sum(a, axis=-1, keepdims=True)
                    return tuple(out_proj(o, wof, r0, ya))
                def pair(i, ya, h0=h0):
                    h = h0 + 2 * i
                    return head1(h + 1, head1(h, ya))
                if n == 2:
                    yacc = pair(0, yacc)
                else:
                    yacc = lax.fori_loop(0, n // 2, pair, yacc)
        with scope("ffn1"):
            attn = jnp.concatenate([jnp.sum(y, axis=0, keepdims=True) for y in yacc], axis=1)
            x = x + attn
            x = ffn(x, wr, wg_s, wu_s, wd_s)
        with scope("attn2"):
            x = attn2(x, kb, vf, wq_s, wof)
        with scope("ffn2"):
            x = ffn(x, wr, wg_s, wu_s, wd_s)
            os_[pl.ds(b, 1), :] = x[0:1, :]
        return carry

    lax.fori_loop(0, _B, batch_body, 0)
    o_ref[...] = os_[0:_B, :].astype(o_ref.dtype)


@jax.jit
def pallas_interleave_layers__sliding_block_cached__moe_arch_mod__decode_kernel(
    A_x, A_k_cache, A_v_cache, A_wq, A_wo, B_x, B_w_r, B_w_gate, B_w_up, B_w_down):
    del B_x
    kt = jnp.transpose(A_k_cache, (0, 1, 3, 2)).reshape(_B, _H * _DH, _SK)
    vt = jnp.transpose(A_v_cache, (0, 1, 3, 2)).reshape(_B, _H * _DH, _SK)
    x2 = A_x.reshape(_B, _D)
    any_spec = pl.BlockSpec(memory_space=pl.ANY)
    vmem_spec = pl.BlockSpec(memory_space=pltpu.VMEM)
    out = pl.pallas_call(
        kernel,
        out_shape=jax.ShapeDtypeStruct((_B, _D), A_x.dtype),
        in_specs=[any_spec] * 9,
        out_specs=vmem_spec,
        scratch_shapes=[
            pltpu.VMEM((2, _NJ, _H * _DH // 2, 128), _U32),
            pltpu.VMEM((2, _NJ, _H * _DH // 2, 128), _U32),
            pltpu.VMEM((_H * _DH // 128, _D // 2, 128), _U32),
            pltpu.VMEM((_H * _DH // 2, _D), _U32),
            pltpu.VMEM((_F // 128, _D // 2, 128), _U32),
            pltpu.VMEM((_F // 128, _D // 2, 128), _U32),
            pltpu.VMEM((_F // 2, _D), _U32),
            pltpu.VMEM((_NJ, _H * _DH, 128), _F32),
            pltpu.VMEM((_H * _DH, _D), _F32),
            pltpu.VMEM((_B, _D), _BF),
            pltpu.VMEM((_D,), _BF),
            pltpu.VMEM((8, _D), _F32),
            pltpu.VMEM((8, _D), _F32),
            pltpu.VMEM((_H, _W), _F32),
            pltpu.SemaphoreType.DMA((2,)),
            pltpu.SemaphoreType.DMA((2, len(V_CHUNKS))),
            pltpu.SemaphoreType.DMA((7,)),
        ],
        compiler_params=pltpu.CompilerParams(vmem_limit_bytes=116 * 1024 * 1024),
    )(x2, B_w_r, kt, vt, A_wq, A_wo, B_w_gate, B_w_up, B_w_down)
    return out.reshape(_B, 1, _D)
```

```python
import functools
import contextlib
import jax
import jax.numpy as jnp
import numpy as np
from jax import lax
import jax.experimental.pallas as pl
import jax.experimental.pallas.tpu as pltpu

_D = 640; _H = 32; _DH = 192; _SK = 4096; _W = 1024; _F = 1536; _B = 4; _NJ = 8
_EPS = 1e-5
_BF = jnp.bfloat16; _F32 = jnp.float32; _U32 = jnp.uint32

V_CHUNKS = [(0, 8), (8, 8), (16, 8), (24, 4), (28, 2), (30, 1), (31, 1)]
GSIZES = (2,) * 16
PROFILE = False

def scope(name):
    return jax.named_scope(name) if PROFILE else contextlib.nullcontext()

def mm(a, b): return jnp.dot(a, b, preferred_element_type=_F32)
def ld(r): return pltpu.bitcast(r, _BF)

def layernorm(x):
    m = jnp.mean(x, axis=-1, keepdims=True)
    xc = x - m
    v = jnp.mean(xc * xc, axis=-1, keepdims=True)
    return xc / jnp.sqrt(v + _EPS)

def bd_mask(gs):
    gd = gs * _DH
    row = lax.broadcasted_iota(jnp.int32, (8, gd), 0)
    col = lax.broadcasted_iota(jnp.int32, (8, gd), 1)
    return (col >= row * _DH) & (col < (row + 1) * _DH)

def softmax_rows(s):
    s = s * (_DH ** -0.5)
    m = jnp.max(s, axis=-1, keepdims=True)
    p = jnp.exp(s - m)
    return p / jnp.sum(p, axis=-1, keepdims=True)

def probs(xn, kb, wq_s, h0, gs):
    gd = gs * _DH
    j0 = h0 * _DH // 128
    q = jnp.concatenate([mm(xn, ld(wq_s[j0 + jj])) for jj in range(gd // 128)], axis=1)
    qbd = jnp.where(bd_mask(gs), q, 0.0).astype(_BF)
    s = jnp.concatenate([mm(qbd, ld(kb[j, h0 * 96:(h0 + gs) * 96, :])) for j in range(_NJ)], axis=1)
    return softmax_rows(s)

def out_proj(o, wof, r0, yacc):
    out = []
    for n in range(_D // 128):
        w = wof[pl.ds(r0, _DH), 128 * n:128 * (n + 1)]
        c = (w * o).reshape(_DH // 8, 8, 128).sum(axis=0)
        out.append(c if yacc is None else yacc[n] + c)
    return out

def tree_sum(ts):
    while len(ts) > 1:
        ts = [ts[i] + ts[i + 1] for i in range(0, len(ts), 2)]
    return ts[0]

def attn2(x, kb, vf, wq_s, wof):
    xn = layernorm(x).astype(_BF)
    ng = len(GSIZES)
    h0s = [sum(GSIZES[:i]) for i in range(ng)]
    qb = {}
    def do_q(gi):
        gs, h0 = GSIZES[gi], h0s[gi]
        nc = gs * _DH // 128; j0 = h0 * _DH // 128
        m = bd_mask(gs)
        qb[gi] = [jnp.where(m[:, 128 * c:128 * (c + 1)], mm(xn, ld(wq_s[j0 + c])), 0.0).astype(_BF) for c in range(nc)]
    yacc = [jnp.zeros((8, 128), _F32)] * (_D // 128)
    do_q(0)
    for gi in range(ng):
        gs, h0 = GSIZES[gi], h0s[gi]
        if gi + 1 < ng: do_q(gi + 1)
        qbd = jnp.concatenate(qb[gi], axis=1)
        s = jnp.concatenate([mm(qbd, ld(kb[j, h0 * 96:(h0 + gs) * 96, :])) for j in range(_NJ)], axis=1)
        p = softmax_rows(s)
        for i in range(gs):
            h = h0 + i
            pb = [jnp.broadcast_to(p[i:i + 1, 128 * j:128 * (j + 1)], (8, 128)) for j in range(_NJ)]
            for r in range(_DH // 8):
                r0 = h * _DH + 8 * r
                ts = [vf[j, r0:r0 + 8, :] * pb[j] for j in range(_NJ)]
                o = jnp.sum(tree_sum(ts), axis=-1, keepdims=True)
                for n in range(_D // 128):
                    yacc[n] = yacc[n] + wof[r0:r0 + 8, 128 * n:128 * (n + 1)] * o
    attn = jnp.concatenate([jnp.sum(y, axis=0, keepdims=True) for y in yacc], axis=1)
    return x + attn

def ffn(x, wr, wg_s, wu_s, wd_s):
    xn = layernorm(x).astype(_BF)
    xnr = xn.astype(_F32)
    r = jnp.sum(xnr * wr, axis=-1, keepdims=True)
    gate = jnp.concatenate([mm(xn, ld(wg_s[jj])) for jj in range(_F // 128)], axis=1)
    up = jnp.concatenate([mm(xn, ld(wu_s[jj])) for jj in range(_F // 128)], axis=1)
    h = (gate * jax.nn.sigmoid(gate) * up).astype(_BF)
    y = jnp.concatenate([mm(h, ld(wd_s[:, 128 * n:128 * (n + 1)])) for n in range(_D // 128)], axis=1)
    return x + (xnr + y * jax.nn.sigmoid(r))

def kernel(x_hbm, wr_hbm, k_hbm, v_hbm, wq_hbm, wo_hbm, wg_hbm, wu_hbm, wd_hbm, o_ref,
           kbuf, vbuf, wq_s, wo_s, wg_s, wu_s, wd_s, vf, wof, x_s, wr_s, xs, os_, ps, ksem, vsem, wsem):
    def k_copy(b, j):
        return pltpu.make_async_copy(k_hbm.at[b, :, pl.ds(pl.multiple_of(_SK - _W + 128 * j, 128), 128)],
                                     kbuf.bitcast(_BF).at[b % 2, j], ksem.at[b % 2])
    def v_copy(b, c, j):
        h0, n = V_CHUNKS[c]
        return pltpu.make_async_copy(v_hbm.at[b, pl.ds(h0 * _DH, n * _DH), pl.ds(pl.multiple_of(_SK - _W + 128 * j, 128), 128)],
                                     vbuf.bitcast(_BF).at[b % 2, j, pl.ds(h0 * _DH, n * _DH)], vsem.at[b % 2, c])
    def w_copy(src, dst, sem_i, j):
        return pltpu.make_async_copy(src.at[:, pl.ds(pl.multiple_of(128 * j, 128), 128)], dst.bitcast(_BF).at[j], wsem.at[sem_i])
    wo_c = pltpu.make_async_copy(wo_hbm, wo_s.bitcast(_BF), wsem.at[1])
    wd_c = pltpu.make_async_copy(wd_hbm, wd_s.bitcast(_BF), wsem.at[4])
    x_c = pltpu.make_async_copy(x_hbm, x_s, wsem.at[5])
    wr_c = pltpu.make_async_copy(wr_hbm, wr_s, wsem.at[6])

    def ordered_starts(n, mk):
        def body(j, c):
            mk(j).start()
            return c
        lax.fori_loop(0, n, body, 0)
    def wait_all(n, mk):
        for j in range(n): mk(j).wait()

    with scope("issue0"):
        ordered_starts(wq_s.shape[0], functools.partial(w_copy, wq_hbm, wq_s, 0))
        x_c.start(); wr_c.start()
        wo_c.start()
        ordered_starts(wg_s.shape[0], functools.partial(w_copy, wg_hbm, wg_s, 2))
        ordered_starts(wu_s.shape[0], functools.partial(w_copy, wu_hbm, wu_s, 3))
        wd_c.start()
        ordered_starts(_NJ, lambda j: k_copy(0, j))
        for c in range(len(V_CHUNKS)):
            ordered_starts(_NJ, lambda j, c=c: v_copy(0, c, j))

    with scope("waitw"):
        x_c.wait(); wr_c.wait()
        xs[...] = jnp.zeros(xs.shape, _F32)
        xs[0:_B, :] = x_s[...].astype(_F32)
        os_[...] = jnp.zeros(os_.shape, _F32)
        wr = wr_s[...].astype(_F32).reshape(1, _D)
        wo_c.wait()
    with scope("mkwof"):
        def unpack_wo(h, c):
            wof[pl.ds(pl.multiple_of(h * _DH, 8), _DH), :] = ld(wo_s[pl.ds(pl.multiple_of(h * 96, 8), 96), :]).astype(_F32)
            return c
        lax.fori_loop(0, _H, unpack_wo, 0)
    with scope("waitw2"):
        wait_all(wq_s.shape[0], functools.partial(w_copy, wq_hbm, wq_s, 0))
        wait_all(wg_s.shape[0], functools.partial(w_copy, wg_hbm, wg_s, 2))
        wait_all(wu_s.shape[0], functools.partial(w_copy, wu_hbm, wu_s, 3))
        wd_c.wait()

    def batch_body(b, carry):
        slot = b % 2
        kb = kbuf.at[slot]; vb = vbuf.at[slot]
        x = jnp.broadcast_to(xs[pl.ds(b, 1), :], (8, _D))
        xn = layernorm(x).astype(_BF)
        with scope("waitk"):
            @pl.when(b + 1 < _B)
            def _():
                ordered_starts(_NJ, lambda j: k_copy(b + 1, j))
            wait_all(_NJ, lambda j: k_copy(b, j))
        with scope("scores1"):
            for g in range(4):
                ps[8 * g:8 * g + 8, :] = probs(xn, kb, wq_s, 8 * g, 8)
        yacc = tuple(jnp.zeros((8, 128), _F32) for _ in range(_D // 128))
        for c, (h0, n) in enumerate(V_CHUNKS):
            with scope(f"waitv{c}"):
                wait_all(_NJ, lambda j, c=c: v_copy(b, c, j))
                @pl.when(b + 1 < _B)
                def _():
                    ordered_starts(_NJ, lambda j, c=c: v_copy(b + 1, c, j))
            with scope(f"pv1_{c}"):
                def head1(h, ya):
                    prow = ps[pl.ds(h, 1), :]
                    pb = [jnp.broadcast_to(prow[:, 128 * j:128 * (j + 1)], (8, 128)) for j in range(_NJ)]
                    ya = list(ya)
                    for r in range(_DH // 16):
                        r0 = pl.multiple_of(h * _DH + 16 * r, 8)
                        w0 = pl.multiple_of(h * 96 + 8 * r, 8)
                        lo = []; hi = []
                        for j in range(_NJ):
                            v = ld(vb[j, pl.ds(w0, 8), :]).astype(_F32)
                            vf[j, pl.ds(r0, 16), :] = v
                            lo.append(v[0:8] * pb[j]); hi.append(v[8:16] * pb[j])
                        for u, ts in enumerate((lo, hi)):
                            o = jnp.sum(tree_sum(ts), axis=-1, keepdims=True)
                            for n in range(_D // 128):
                                ya[n] = ya[n] + wof[pl.ds(r0 + 8 * u, 8), 128 * n:128 * (n + 1)] * o
                    return tuple(ya)
                def pair(i, ya, h0=h0):
                    h = h0 + 2 * i
                    return head1(h + 1, head1(h, ya))
                if n == 1:
                    yacc = head1(h0, yacc)
                elif n == 2:
                    yacc = pair(0, yacc)
                else:
                    yacc = lax.fori_loop(0, n // 2, pair, yacc)
        with scope("ffn1"):
            attn = jnp.concatenate([jnp.sum(y, axis=0, keepdims=True) for y in yacc], axis=1)
            x = x + attn
            x = ffn(x, wr, wg_s, wu_s, wd_s)
        with scope("attn2"):
            x = attn2(x, kb, vf, wq_s, wof)
        with scope("ffn2"):
            x = ffn(x, wr, wg_s, wu_s, wd_s)
            os_[pl.ds(b, 1), :] = x[0:1, :]
        return carry

    lax.fori_loop(0, _B, batch_body, 0)
    o_ref[...] = os_[0:_B, :].astype(o_ref.dtype)


@jax.jit
def pallas_interleave_layers__sliding_block_cached__moe_arch_mod__decode_kernel(
    A_x, A_k_cache, A_v_cache, A_wq, A_wo, B_x, B_w_r, B_w_gate, B_w_up, B_w_down):
    del B_x
    kt = jnp.transpose(A_k_cache, (0, 1, 3, 2)).reshape(_B, _H * _DH, _SK)
    vt = jnp.transpose(A_v_cache, (0, 1, 3, 2)).reshape(_B, _H * _DH, _SK)
    x2 = A_x.reshape(_B, _D)
    any_spec = pl.BlockSpec(memory_space=pl.ANY)
    vmem_spec = pl.BlockSpec(memory_space=pltpu.VMEM)
    out = pl.pallas_call(
        kernel,
        out_shape=jax.ShapeDtypeStruct((_B, _D), A_x.dtype),
        in_specs=[any_spec] * 9,
        out_specs=vmem_spec,
        scratch_shapes=[
            pltpu.VMEM((2, _NJ, _H * _DH // 2, 128), _U32),
            pltpu.VMEM((2, _NJ, _H * _DH // 2, 128), _U32),
            pltpu.VMEM((_H * _DH // 128, _D // 2, 128), _U32),
            pltpu.VMEM((_H * _DH // 2, _D), _U32),
            pltpu.VMEM((_F // 128, _D // 2, 128), _U32),
            pltpu.VMEM((_F // 128, _D // 2, 128), _U32),
            pltpu.VMEM((_F // 2, _D), _U32),
            pltpu.VMEM((_NJ, _H * _DH, 128), _F32),
            pltpu.VMEM((_H * _DH, _D), _F32),
            pltpu.VMEM((_B, _D), _BF),
            pltpu.VMEM((_D,), _BF),
            pltpu.VMEM((8, _D), _F32),
            pltpu.VMEM((8, _D), _F32),
            pltpu.VMEM((_H, _W), _F32),
            pltpu.SemaphoreType.DMA((2,)),
            pltpu.SemaphoreType.DMA((2, len(V_CHUNKS))),
            pltpu.SemaphoreType.DMA((7,)),
        ],
        compiler_params=pltpu.CompilerParams(vmem_limit_bytes=116 * 1024 * 1024),
    )(x2, B_w_r, kt, vt, A_wq, A_wo, B_w_gate, B_w_up, B_w_down)
    return out.reshape(_B, 1, _D)
```

```python
import functools
import contextlib
import jax
import jax.numpy as jnp
import numpy as np
from jax import lax
import jax.experimental.pallas as pl
import jax.experimental.pallas.tpu as pltpu

_D = 640; _H = 32; _DH = 192; _SK = 4096; _W = 1024; _F = 1536; _B = 4; _NJ = 8
_EPS = 1e-5
_BF = jnp.bfloat16; _F32 = jnp.float32; _U32 = jnp.uint32

V_CHUNKS = [(0, 8), (8, 8), (16, 8), (24, 4), (28, 2), (30, 1), (31, 1)]
GSIZES = (2,) * 16
PROFILE = False

def scope(name):
    return jax.named_scope(name) if PROFILE else contextlib.nullcontext()

def mm(a, b): return jnp.dot(a, b, preferred_element_type=_F32)
def ld(r): return pltpu.bitcast(r, _BF)

def layernorm(x):
    m = jnp.mean(x, axis=-1, keepdims=True)
    xc = x - m
    v = jnp.mean(xc * xc, axis=-1, keepdims=True)
    return xc / jnp.sqrt(v + _EPS)

def ln_parts(x):
    xc = x - jnp.mean(x, axis=-1, keepdims=True)
    v = jnp.mean(xc * xc, axis=-1, keepdims=True)
    return xc, lax.rsqrt(v + _EPS)

def bd_mask(gs):
    gd = gs * _DH
    row = lax.broadcasted_iota(jnp.int32, (8, gd), 0)
    col = lax.broadcasted_iota(jnp.int32, (8, gd), 1)
    return (col >= row * _DH) & (col < (row + 1) * _DH)

def softmax_rows(s):
    s = s * (_DH ** -0.5)
    m = jnp.max(s, axis=-1, keepdims=True)
    p = jnp.exp(s - m)
    return p / jnp.sum(p, axis=-1, keepdims=True)

def probs(xn, kb, wq_s, h0, gs):
    gd = gs * _DH
    j0 = h0 * _DH // 128
    q = jnp.concatenate([mm(xn, ld(wq_s[j0 + jj])) for jj in range(gd // 128)], axis=1)
    qbd = jnp.where(bd_mask(gs), q, 0.0).astype(_BF)
    s = jnp.concatenate([mm(qbd, ld(kb[j, h0 * 96:(h0 + gs) * 96, :])) for j in range(_NJ)], axis=1)
    return softmax_rows(s)

def out_proj(o, wof, r0, yacc):
    out = []
    for n in range(_D // 128):
        w = wof[pl.ds(r0, _DH), 128 * n:128 * (n + 1)]
        c = (w * o).reshape(_DH // 8, 8, 128).sum(axis=0)
        out.append(c if yacc is None else yacc[n] + c)
    return out

def tree_sum(ts):
    while len(ts) > 1:
        ts = [ts[i] + ts[i + 1] for i in range(0, len(ts), 2)]
    return ts[0]

def attn2(x, kb, vf, wq_s, wof):
    xc, rstd = ln_parts(x)
    xn = xc.astype(_BF)
    ng = len(GSIZES)
    h0s = [sum(GSIZES[:i]) for i in range(ng)]
    qb = {}
    def do_q(gi):
        gs, h0 = GSIZES[gi], h0s[gi]
        nc = gs * _DH // 128; j0 = h0 * _DH // 128
        m = bd_mask(gs)
        qb[gi] = [jnp.where(m[:, 128 * c:128 * (c + 1)], mm(xn, ld(wq_s[j0 + c])) * rstd, 0.0).astype(_BF) for c in range(nc)]
    yacc = [jnp.zeros((8, 128), _F32)] * (_D // 128)
    do_q(0)
    for gi in range(ng):
        gs, h0 = GSIZES[gi], h0s[gi]
        if gi + 1 < ng: do_q(gi + 1)
        qbd = jnp.concatenate(qb[gi], axis=1)
        s = jnp.concatenate([mm(qbd, ld(kb[j, h0 * 96:(h0 + gs) * 96, :])) for j in range(_NJ)], axis=1)
        p = softmax_rows(s)
        for i in range(gs):
            h = h0 + i
            pb = [jnp.broadcast_to(p[i:i + 1, 128 * j:128 * (j + 1)], (8, 128)) for j in range(_NJ)]
            for r in range(_DH // 8):
                r0 = h * _DH + 8 * r
                ts = [vf[j, r0:r0 + 8, :] * pb[j] for j in range(_NJ)]
                o = jnp.sum(tree_sum(ts), axis=-1, keepdims=True)
                for n in range(_D // 128):
                    yacc[n] = yacc[n] + wof[r0:r0 + 8, 128 * n:128 * (n + 1)] * o
    attn = jnp.concatenate([jnp.sum(y, axis=0, keepdims=True) for y in yacc], axis=1)
    return x + attn

NV = 3

def ffn(x, wr, wg_s, wu_s, wd_s, wgu_f):
    xc, rstd = ln_parts(x)
    xn = xc.astype(_BF)
    xnr = xn.astype(_F32)
    r = jnp.sum(xnr * wr, axis=-1, keepdims=True) * rstd
    nm = _F // 128 - NV
    gate = [mm(xn, ld(wg_s[jj])) for jj in range(nm)]
    up = [mm(xn, ld(wu_s[jj])) for jj in range(nm)]
    if NV:
        xb = jnp.concatenate([jnp.broadcast_to(xnr[0:1, 128 * i:128 * (i + 1)], (128, 128)).T
                              for i in range(_D // 128)], axis=0)
        acc = [None] * (2 * NV)
        for kc in range(_D // 16):
            x2 = xb[16 * kc:16 * kc + 16]
            for i in range(2 * NV):
                t = wgu_f[i, 16 * kc:16 * kc + 16, :] * x2
                t = t[0:8] + t[8:16]
                acc[i] = t if acc[i] is None else acc[i] + t
        fin = lambda c: jnp.broadcast_to(jnp.sum(c, axis=0, keepdims=True), (8, 128))
        gate += [fin(c) for c in acc[:NV]]
        up += [fin(c) for c in acc[NV:]]
    gate = jnp.concatenate(gate, axis=1) * rstd
    up = jnp.concatenate(up, axis=1) * rstd
    h = (gate * jax.nn.sigmoid(gate) * up).astype(_BF)
    y = jnp.concatenate([mm(h, ld(wd_s[:, 128 * n:128 * (n + 1)])) for n in range(_D // 128)], axis=1)
    return x + (xc * rstd + y * jax.nn.sigmoid(r))

def kernel(x_hbm, wr_hbm, k_hbm, v_hbm, wq_hbm, wo_hbm, wg_hbm, wu_hbm, wd_hbm, o_ref,
           kbuf, vbuf, wq_s, wo_s, wg_s, wu_s, wd_s, vf, wof, wgu_f, x_s, wr_s, xs, os_, ps, ksem, vsem, wsem):
    def k_copy(b, j):
        return pltpu.make_async_copy(k_hbm.at[b, :, pl.ds(pl.multiple_of(_SK - _W + 128 * j, 128), 128)],
                                     kbuf.bitcast(_BF).at[b % 2, j], ksem.at[b % 2])
    def v_copy(b, c, j):
        h0, n = V_CHUNKS[c]
        return pltpu.make_async_copy(v_hbm.at[b, pl.ds(h0 * _DH, n * _DH), pl.ds(pl.multiple_of(_SK - _W + 128 * j, 128), 128)],
                                     vbuf.bitcast(_BF).at[b % 2, j, pl.ds(h0 * _DH, n * _DH)], vsem.at[b % 2, c])
    def w_copy(src, dst, sem_i, j):
        return pltpu.make_async_copy(src.at[:, pl.ds(pl.multiple_of(128 * j, 128), 128)], dst.bitcast(_BF).at[j], wsem.at[sem_i])
    wo_c = pltpu.make_async_copy(wo_hbm, wo_s.bitcast(_BF), wsem.at[1])
    wd_c = pltpu.make_async_copy(wd_hbm, wd_s.bitcast(_BF), wsem.at[4])
    x_c = pltpu.make_async_copy(x_hbm, x_s, wsem.at[5])
    wr_c = pltpu.make_async_copy(wr_hbm, wr_s, wsem.at[6])

    def ordered_starts(n, mk):
        def body(j, c):
            mk(j).start()
            return c
        lax.fori_loop(0, n, body, 0)
    def wait_all(n, mk):
        for j in range(n): mk(j).wait()

    with scope("issue0"):
        ordered_starts(wq_s.shape[0], functools.partial(w_copy, wq_hbm, wq_s, 0))
        x_c.start(); wr_c.start()
        wo_c.start()
        ordered_starts(wg_s.shape[0], functools.partial(w_copy, wg_hbm, wg_s, 2))
        ordered_starts(wu_s.shape[0], functools.partial(w_copy, wu_hbm, wu_s, 3))
        wd_c.start()
        ordered_starts(_NJ, lambda j: k_copy(0, j))
        for c in range(len(V_CHUNKS)):
            ordered_starts(_NJ, lambda j, c=c: v_copy(0, c, j))

    with scope("waitw"):
        x_c.wait(); wr_c.wait()
        xs[...] = jnp.zeros(xs.shape, _F32)
        xs[0:_B, :] = x_s[...].astype(_F32)
        os_[...] = jnp.zeros(os_.shape, _F32)
        wr = wr_s[...].astype(_F32).reshape(1, _D)
        wo_c.wait()
    with scope("mkwof"):
        def unpack_wo(h, c):
            wof[pl.ds(pl.multiple_of(h * _DH, 8), _DH), :] = ld(wo_s[pl.ds(pl.multiple_of(h * 96, 8), 96), :]).astype(_F32)
            return c
        lax.fori_loop(0, _H, unpack_wo, 0)
    with scope("waitw2"):
        wait_all(wq_s.shape[0], functools.partial(w_copy, wq_hbm, wq_s, 0))
        wait_all(wg_s.shape[0], functools.partial(w_copy, wg_hbm, wg_s, 2))
        wait_all(wu_s.shape[0], functools.partial(w_copy, wu_hbm, wu_s, 3))
        wd_c.wait()
        for i in range(NV):
            wgu_f[i] = ld(wg_s[_F // 128 - NV + i]).astype(_F32)
            wgu_f[NV + i] = ld(wu_s[_F // 128 - NV + i]).astype(_F32)

    def batch_body(b, carry):
        slot = b % 2
        kb = kbuf.at[slot]; vb = vbuf.at[slot]
        x = jnp.broadcast_to(xs[pl.ds(b, 1), :], (8, _D))
        xn = layernorm(x).astype(_BF)
        with scope("waitk"):
            @pl.when(b + 1 < _B)
            def _():
                ordered_starts(_NJ, lambda j: k_copy(b + 1, j))
            wait_all(_NJ, lambda j: k_copy(b, j))
        with scope("scores1"):
            for g in range(4):
                ps[8 * g:8 * g + 8, :] = probs(xn, kb, wq_s, 8 * g, 8)
        yacc = tuple(jnp.zeros((8, 128), _F32) for _ in range(_D // 128))
        for c, (h0, n) in enumerate(V_CHUNKS):
            with scope(f"waitv{c}"):
                wait_all(_NJ, lambda j, c=c: v_copy(b, c, j))
                @pl.when(b + 1 < _B)
                def _():
                    ordered_starts(_NJ, lambda j, c=c: v_copy(b + 1, c, j))
            with scope(f"pv1_{c}"):
                def head1(h, ya):
                    prow = ps[pl.ds(h, 1), :]
                    pb = [jnp.broadcast_to(prow[:, 128 * j:128 * (j + 1)], (8, 128)) for j in range(_NJ)]
                    ya = list(ya)
                    for r in range(_DH // 16):
                        r0 = pl.multiple_of(h * _DH + 16 * r, 8)
                        w0 = pl.multiple_of(h * 96 + 8 * r, 8)
                        lo = []; hi = []
                        for j in range(_NJ):
                            v = ld(vb[j, pl.ds(w0, 8), :]).astype(_F32)
                            vf[j, pl.ds(r0, 16), :] = v
                            lo.append(v[0:8] * pb[j]); hi.append(v[8:16] * pb[j])
                        for u, ts in enumerate((lo, hi)):
                            o = jnp.sum(tree_sum(ts), axis=-1, keepdims=True)
                            for n in range(_D // 128):
                                ya[n] = ya[n] + wof[pl.ds(r0 + 8 * u, 8), 128 * n:128 * (n + 1)] * o
                    return tuple(ya)
                def pair(i, ya, h0=h0):
                    h = h0 + 2 * i
                    return head1(h + 1, head1(h, ya))
                if n == 1:
                    yacc = head1(h0, yacc)
                elif n == 2:
                    yacc = pair(0, yacc)
                else:
                    yacc = lax.fori_loop(0, n // 2, pair, yacc)
        with scope("ffn1"):
            attn = jnp.concatenate([jnp.sum(y, axis=0, keepdims=True) for y in yacc], axis=1)
            x = x + attn
            x = ffn(x, wr, wg_s, wu_s, wd_s, wgu_f)
        with scope("attn2"):
            x = attn2(x, kb, vf, wq_s, wof)
        with scope("ffn2"):
            x = ffn(x, wr, wg_s, wu_s, wd_s, wgu_f)
            os_[pl.ds(b, 1), :] = x[0:1, :]
        return carry

    lax.fori_loop(0, _B, batch_body, 0)
    o_ref[...] = os_[0:_B, :].astype(o_ref.dtype)


@jax.jit
def pallas_interleave_layers__sliding_block_cached__moe_arch_mod__decode_kernel(
    A_x, A_k_cache, A_v_cache, A_wq, A_wo, B_x, B_w_r, B_w_gate, B_w_up, B_w_down):
    del B_x
    kt = jnp.transpose(A_k_cache, (0, 1, 3, 2)).reshape(_B, _H * _DH, _SK)
    vt = jnp.transpose(A_v_cache, (0, 1, 3, 2)).reshape(_B, _H * _DH, _SK)
    x2 = A_x.reshape(_B, _D)
    any_spec = pl.BlockSpec(memory_space=pl.ANY)
    vmem_spec = pl.BlockSpec(memory_space=pltpu.VMEM)
    out = pl.pallas_call(
        kernel,
        out_shape=jax.ShapeDtypeStruct((_B, _D), A_x.dtype),
        in_specs=[any_spec] * 9,
        out_specs=vmem_spec,
        scratch_shapes=[
            pltpu.VMEM((2, _NJ, _H * _DH // 2, 128), _U32),
            pltpu.VMEM((2, _NJ, _H * _DH // 2, 128), _U32),
            pltpu.VMEM((_H * _DH // 128, _D // 2, 128), _U32),
            pltpu.VMEM((_H * _DH // 2, _D), _U32),
            pltpu.VMEM((_F // 128, _D // 2, 128), _U32),
            pltpu.VMEM((_F // 128, _D // 2, 128), _U32),
            pltpu.VMEM((_F // 2, _D), _U32),
            pltpu.VMEM((_NJ, _H * _DH, 128), _F32),
            pltpu.VMEM((_H * _DH, _D), _F32),
            pltpu.VMEM((max(2 * NV, 1), _D, 128), _F32),
            pltpu.VMEM((_B, _D), _BF),
            pltpu.VMEM((_D,), _BF),
            pltpu.VMEM((8, _D), _F32),
            pltpu.VMEM((8, _D), _F32),
            pltpu.VMEM((_H, _W), _F32),
            pltpu.SemaphoreType.DMA((2,)),
            pltpu.SemaphoreType.DMA((2, len(V_CHUNKS))),
            pltpu.SemaphoreType.DMA((7,)),
        ],
        compiler_params=pltpu.CompilerParams(vmem_limit_bytes=116 * 1024 * 1024),
    )(x2, B_w_r, kt, vt, A_wq, A_wo, B_w_gate, B_w_up, B_w_down)
    return out.reshape(_B, 1, _D)
```

```python
import functools
import contextlib
import jax
import jax.numpy as jnp
import numpy as np
from jax import lax
import jax.experimental.pallas as pl
import jax.experimental.pallas.tpu as pltpu

_D = 640; _H = 32; _DH = 192; _SK = 4096; _W = 1024; _F = 1536; _B = 4; _NJ = 8
_EPS = 1e-5
_BF = jnp.bfloat16; _F32 = jnp.float32; _U32 = jnp.uint32

V_CHUNKS = [(0, 8), (8, 8), (16, 8), (24, 4), (28, 2), (30, 1), (31, 1)]
GSIZES = (2,) * 16
PROFILE = False

def scope(name):
    return jax.named_scope(name) if PROFILE else contextlib.nullcontext()

def mm(a, b): return jnp.dot(a, b, preferred_element_type=_F32)
def ld(r): return pltpu.bitcast(r, _BF)

def layernorm(x):
    m = jnp.mean(x, axis=-1, keepdims=True)
    xc = x - m
    v = jnp.mean(xc * xc, axis=-1, keepdims=True)
    return xc / jnp.sqrt(v + _EPS)

def ln_parts(x):
    xc = x - jnp.mean(x, axis=-1, keepdims=True)
    v = jnp.mean(xc * xc, axis=-1, keepdims=True)
    return xc, lax.rsqrt(v + _EPS)

def bd_mask(gs):
    gd = gs * _DH
    row = lax.broadcasted_iota(jnp.int32, (8, gd), 0)
    col = lax.broadcasted_iota(jnp.int32, (8, gd), 1)
    return (col >= row * _DH) & (col < (row + 1) * _DH)

_QSCALE = float(_DH ** -0.5 * np.log2(np.e))

def softmax_rows(s):
    m = jnp.max(s, axis=-1, keepdims=True)
    p = jnp.exp2(s - m)
    return p * (1.0 / jnp.sum(p, axis=-1, keepdims=True))

def probs(xn, kb, wq_s, h0, gs):
    gd = gs * _DH
    j0 = h0 * _DH // 128
    q = jnp.concatenate([mm(xn, ld(wq_s[j0 + jj])) for jj in range(gd // 128)], axis=1)
    qbd = jnp.where(bd_mask(gs), q * _QSCALE, 0.0).astype(_BF)
    s = jnp.concatenate([mm(qbd, ld(kb[j, h0 * 96:(h0 + gs) * 96, :])) for j in range(_NJ)], axis=1)
    return softmax_rows(s)

def out_proj(o, wof, r0, yacc):
    out = []
    for n in range(_D // 128):
        w = wof[pl.ds(r0, _DH), 128 * n:128 * (n + 1)]
        c = (w * o).reshape(_DH // 8, 8, 128).sum(axis=0)
        out.append(c if yacc is None else yacc[n] + c)
    return out

def tree_sum(ts):
    while len(ts) > 1:
        ts = [ts[i] + ts[i + 1] for i in range(0, len(ts), 2)]
    return ts[0]

def attn2(x, kb, vf, wq_s, wof):
    xc, rstd = ln_parts(x)
    xn = xc.astype(_BF)
    qs = rstd * _QSCALE
    ng = len(GSIZES)
    h0s = [sum(GSIZES[:i]) for i in range(ng)]
    qb = {}
    def do_q(gi):
        gs, h0 = GSIZES[gi], h0s[gi]
        nc = gs * _DH // 128; j0 = h0 * _DH // 128
        m = bd_mask(gs)
        qb[gi] = [jnp.where(m[:, 128 * c:128 * (c + 1)], mm(xn, ld(wq_s[j0 + c])) * qs, 0.0).astype(_BF) for c in range(nc)]
    yacc = [jnp.zeros((8, 128), _F32)] * (_D // 128)
    do_q(0)
    for gi in range(ng):
        gs, h0 = GSIZES[gi], h0s[gi]
        if gi + 1 < ng: do_q(gi + 1)
        qbd = jnp.concatenate(qb[gi], axis=1)
        s = jnp.concatenate([mm(qbd, ld(kb[j, h0 * 96:(h0 + gs) * 96, :])) for j in range(_NJ)], axis=1)
        p = softmax_rows(s)
        for i in range(gs):
            h = h0 + i
            pb = [jnp.broadcast_to(p[i:i + 1, 128 * j:128 * (j + 1)], (8, 128)) for j in range(_NJ)]
            for r in range(_DH // 8):
                r0 = h * _DH + 8 * r
                ts = [vf[j, r0:r0 + 8, :] * pb[j] for j in range(_NJ)]
                o = jnp.sum(tree_sum(ts), axis=-1, keepdims=True)
                for n in range(_D // 128):
                    yacc[n] = yacc[n] + wof[r0:r0 + 8, 128 * n:128 * (n + 1)] * o
    attn = jnp.concatenate([jnp.sum(y, axis=0, keepdims=True) for y in yacc], axis=1)
    return x + attn

NV = 2
KD = 8

def col_bcast(row):
    return jnp.broadcast_to(row, (128, 128)).T

def rows_total(c):
    return jnp.broadcast_to(jnp.sum(c, axis=0, keepdims=True), (8, 128))

def ffn(x, wr, wg_s, wu_s, wd_s, wgu_f, wd_f):
    xc, rstd = ln_parts(x)
    xn = xc.astype(_BF)
    xnr = xn.astype(_F32)
    r = jnp.sum(xnr * wr, axis=-1, keepdims=True) * rstd
    nf = _F // 128
    nm = nf - NV
    nd = _D // 128
    gate = [None] * nf
    up = [None] * nf
    for jj in range(nm):
        gate[jj] = mm(xn, ld(wg_s[jj]))
        up[jj] = mm(xn, ld(wu_s[jj]))
    xb = jnp.concatenate([col_bcast(xnr[0:1, 128 * i:128 * (i + 1)]) for i in range(nd)], axis=0)
    acc = [None] * (2 * NV)
    for kc in range(_D // 16):
        x2 = xb[16 * kc:16 * kc + 16]
        for i in range(2 * NV):
            t = wgu_f[i, 16 * kc:16 * kc + 16, :] * x2
            t = t[0:8] + t[8:16]
            acc[i] = t if acc[i] is None else acc[i] + t
    for i in range(NV):
        gate[nm + i] = rows_total(acc[i])
        up[nm + i] = rows_total(acc[NV + i])
    hs = []
    for jj in range(nf):
        g = gate[jj] * rstd
        hs.append((g * jax.nn.sigmoid(g) * (up[jj] * rstd)).astype(_BF))
    hm = jnp.concatenate(hs[KD:], axis=1)
    y = jnp.concatenate([mm(hm, ld(wd_s[64 * KD:, 128 * n:128 * (n + 1)])) for n in range(nd)], axis=1)
    ya = [None] * nd
    for blk in range(KD):
        hb = col_bcast(hs[blk].astype(_F32)[0:1, :])
        for rr in range(16):
            h2 = hb[8 * rr:8 * rr + 8]
            r0 = 128 * blk + 8 * rr
            for n in range(nd):
                t = wd_f[r0:r0 + 8, 128 * n:128 * (n + 1)] * h2
                ya[n] = t if ya[n] is None else ya[n] + t
    y = y + jnp.concatenate([rows_total(c) for c in ya], axis=1)
    return x + (xc * rstd + y * jax.nn.sigmoid(r))

def kernel(x_hbm, wr_hbm, k_hbm, v_hbm, wq_hbm, wo_hbm, wg_hbm, wu_hbm, wd_hbm, o_ref,
           kbuf, vbuf, wq_s, wo_s, wg_s, wu_s, wd_s, vf, wof, wgu_f, wd_f, x_s, wr_s, xs, os_, ps, ksem, vsem, wsem):
    def k_copy(b, j):
        return pltpu.make_async_copy(k_hbm.at[b, :, pl.ds(pl.multiple_of(_SK - _W + 128 * j, 128), 128)],
                                     kbuf.bitcast(_BF).at[b % 2, j], ksem.at[b % 2])
    def v_copy(b, c, j):
        h0, n = V_CHUNKS[c]
        return pltpu.make_async_copy(v_hbm.at[b, pl.ds(h0 * _DH, n * _DH), pl.ds(pl.multiple_of(_SK - _W + 128 * j, 128), 128)],
                                     vbuf.bitcast(_BF).at[b % 2, j, pl.ds(h0 * _DH, n * _DH)], vsem.at[b % 2, c])
    def w_copy(src, dst, sem_i, j):
        return pltpu.make_async_copy(src.at[:, pl.ds(pl.multiple_of(128 * j, 128), 128)], dst.bitcast(_BF).at[j], wsem.at[sem_i])
    wo_c = pltpu.make_async_copy(wo_hbm, wo_s.bitcast(_BF), wsem.at[1])
    wd_c = pltpu.make_async_copy(wd_hbm, wd_s.bitcast(_BF), wsem.at[4])
    x_c = pltpu.make_async_copy(x_hbm, x_s, wsem.at[5])
    wr_c = pltpu.make_async_copy(wr_hbm, wr_s, wsem.at[6])

    def ordered_starts(n, mk):
        def body(j, c):
            mk(j).start()
            return c
        lax.fori_loop(0, n, body, 0)
    def wait_all(n, mk):
        for j in range(n): mk(j).wait()

    with scope("issue0"):
        ordered_starts(wq_s.shape[0], functools.partial(w_copy, wq_hbm, wq_s, 0))
        x_c.start(); wr_c.start()
        wo_c.start()
        ordered_starts(wg_s.shape[0], functools.partial(w_copy, wg_hbm, wg_s, 2))
        ordered_starts(wu_s.shape[0], functools.partial(w_copy, wu_hbm, wu_s, 3))
        wd_c.start()
        ordered_starts(_NJ, lambda j: k_copy(0, j))
        for c in range(len(V_CHUNKS)):
            ordered_starts(_NJ, lambda j, c=c: v_copy(0, c, j))

    with scope("waitw"):
        x_c.wait(); wr_c.wait()
        xs[...] = jnp.zeros(xs.shape, _F32)
        xs[0:_B, :] = x_s[...].astype(_F32)
        os_[...] = jnp.zeros(os_.shape, _F32)
        wr = wr_s[...].astype(_F32).reshape(1, _D)
        wo_c.wait()
    with scope("mkwof"):
        def unpack_wo(h, c):
            wof[pl.ds(pl.multiple_of(h * _DH, 8), _DH), :] = ld(wo_s[pl.ds(pl.multiple_of(h * 96, 8), 96), :]).astype(_F32)
            return c
        lax.fori_loop(0, _H, unpack_wo, 0)
    with scope("waitw2"):
        wait_all(wq_s.shape[0], functools.partial(w_copy, wq_hbm, wq_s, 0))
        wait_all(wg_s.shape[0], functools.partial(w_copy, wg_hbm, wg_s, 2))
        wait_all(wu_s.shape[0], functools.partial(w_copy, wu_hbm, wu_s, 3))
        wd_c.wait()
        for i in range(NV):
            wgu_f[i] = ld(wg_s[_F // 128 - NV + i]).astype(_F32)
            wgu_f[NV + i] = ld(wu_s[_F // 128 - NV + i]).astype(_F32)
        for blk in range(KD):
            wd_f[128 * blk:128 * (blk + 1), :] = ld(wd_s[64 * blk:64 * (blk + 1), :]).astype(_F32)

    def batch_body(b, carry):
        slot = b % 2
        kb = kbuf.at[slot]; vb = vbuf.at[slot]
        x = jnp.broadcast_to(xs[pl.ds(b, 1), :], (8, _D))
        xn = layernorm(x).astype(_BF)
        with scope("waitk"):
            @pl.when(b + 1 < _B)
            def _():
                ordered_starts(_NJ, lambda j: k_copy(b + 1, j))
            wait_all(_NJ, lambda j: k_copy(b, j))
        with scope("scores1"):
            for g in range(4):
                ps[8 * g:8 * g + 8, :] = probs(xn, kb, wq_s, 8 * g, 8)
        yacc = tuple(jnp.zeros((8, 128), _F32) for _ in range(_D // 128))
        for c, (h0, n) in enumerate(V_CHUNKS):
            with scope(f"waitv{c}"):
                wait_all(_NJ, lambda j, c=c: v_copy(b, c, j))
                @pl.when(b + 1 < _B)
                def _():
                    ordered_starts(_NJ, lambda j, c=c: v_copy(b + 1, c, j))
            with scope(f"pv1_{c}"):
                def head1(h, ya):
                    prow = ps[pl.ds(h, 1), :]
                    pb = [jnp.broadcast_to(prow[:, 128 * j:128 * (j + 1)], (8, 128)) for j in range(_NJ)]
                    ya = list(ya)
                    for r in range(_DH // 16):
                        r0 = pl.multiple_of(h * _DH + 16 * r, 8)
                        w0 = pl.multiple_of(h * 96 + 8 * r, 8)
                        lo = []; hi = []
                        for j in range(_NJ):
                            v = ld(vb[j, pl.ds(w0, 8), :]).astype(_F32)
                            vf[j, pl.ds(r0, 16), :] = v
                            lo.append(v[0:8] * pb[j]); hi.append(v[8:16] * pb[j])
                        for u, ts in enumerate((lo, hi)):
                            o = jnp.sum(tree_sum(ts), axis=-1, keepdims=True)
                            for n in range(_D // 128):
                                ya[n] = ya[n] + wof[pl.ds(r0 + 8 * u, 8), 128 * n:128 * (n + 1)] * o
                    return tuple(ya)
                def pair(i, ya, h0=h0):
                    h = h0 + 2 * i
                    return head1(h + 1, head1(h, ya))
                if n == 1:
                    yacc = head1(h0, yacc)
                elif n == 2:
                    yacc = pair(0, yacc)
                else:
                    yacc = lax.fori_loop(0, n // 2, pair, yacc)
        with scope("ffn1"):
            attn = jnp.concatenate([jnp.sum(y, axis=0, keepdims=True) for y in yacc], axis=1)
            x = x + attn
            x = ffn(x, wr, wg_s, wu_s, wd_s, wgu_f, wd_f)
        with scope("attn2"):
            x = attn2(x, kb, vf, wq_s, wof)
        with scope("ffn2"):
            x = ffn(x, wr, wg_s, wu_s, wd_s, wgu_f, wd_f)
            os_[pl.ds(b, 1), :] = x[0:1, :]
        return carry

    lax.fori_loop(0, _B, batch_body, 0)
    o_ref[...] = os_[0:_B, :].astype(o_ref.dtype)


@jax.jit
def pallas_interleave_layers__sliding_block_cached__moe_arch_mod__decode_kernel(
    A_x, A_k_cache, A_v_cache, A_wq, A_wo, B_x, B_w_r, B_w_gate, B_w_up, B_w_down):
    del B_x
    kt = jnp.transpose(A_k_cache, (0, 1, 3, 2)).reshape(_B, _H * _DH, _SK)
    vt = jnp.transpose(A_v_cache, (0, 1, 3, 2)).reshape(_B, _H * _DH, _SK)
    x2 = A_x.reshape(_B, _D)
    any_spec = pl.BlockSpec(memory_space=pl.ANY)
    vmem_spec = pl.BlockSpec(memory_space=pltpu.VMEM)
    out = pl.pallas_call(
        kernel,
        out_shape=jax.ShapeDtypeStruct((_B, _D), A_x.dtype),
        in_specs=[any_spec] * 9,
        out_specs=vmem_spec,
        scratch_shapes=[
            pltpu.VMEM((2, _NJ, _H * _DH // 2, 128), _U32),
            pltpu.VMEM((2, _NJ, _H * _DH // 2, 128), _U32),
            pltpu.VMEM((_H * _DH // 128, _D // 2, 128), _U32),
            pltpu.VMEM((_H * _DH // 2, _D), _U32),
            pltpu.VMEM((_F // 128, _D // 2, 128), _U32),
            pltpu.VMEM((_F // 128, _D // 2, 128), _U32),
            pltpu.VMEM((_F // 2, _D), _U32),
            pltpu.VMEM((_NJ, _H * _DH, 128), _F32),
            pltpu.VMEM((_H * _DH, _D), _F32),
            pltpu.VMEM((2 * NV, _D, 128), _F32),
            pltpu.VMEM((128 * KD, _D), _F32),
            pltpu.VMEM((_B, _D), _BF),
            pltpu.VMEM((_D,), _BF),
            pltpu.VMEM((8, _D), _F32),
            pltpu.VMEM((8, _D), _F32),
            pltpu.VMEM((_H, _W), _F32),
            pltpu.SemaphoreType.DMA((2,)),
            pltpu.SemaphoreType.DMA((2, len(V_CHUNKS))),
            pltpu.SemaphoreType.DMA((7,)),
        ],
        compiler_params=pltpu.CompilerParams(vmem_limit_bytes=116 * 1024 * 1024),
    )(x2, B_w_r, kt, vt, A_wq, A_wo, B_w_gate, B_w_up, B_w_down)
    return out.reshape(_B, 1, _D)
```

```python
import functools

import jax
import jax.numpy as jnp
import numpy as np
from jax import lax
import jax.experimental.pallas as pl
import jax.experimental.pallas.tpu as pltpu

_D = 640
_H = 32
_DH = 192
_SK = 4096
_W = 1024
_F = 1536
_B = 4
_NJ = _W // 128
_ND = _D // 128
_EPS = 1e-5
_BF = jnp.bfloat16
_F32 = jnp.float32
_U32 = jnp.uint32

_V_CHUNKS = ((0, 8), (8, 8), (16, 8), (24, 4), (28, 2), (30, 1), (31, 1))
_GS = 2
_LAG = 4
_NV = 2
_KD = 8
_QSCALE = float(_DH ** -0.5 * np.log2(np.e))


def _mm(a, b):
    return jnp.dot(a, b, preferred_element_type=_F32)


def _ld(words):
    return pltpu.bitcast(words, _BF)


def _ln_parts(x):
    xc = x - jnp.mean(x, axis=-1, keepdims=True)
    var = jnp.mean(xc * xc, axis=-1, keepdims=True)
    return xc, lax.rsqrt(var + _EPS)


def _head_mask(gs):
    row = lax.broadcasted_iota(jnp.int32, (8, gs * _DH), 0)
    col = lax.broadcasted_iota(jnp.int32, (8, gs * _DH), 1)
    return (col >= row * _DH) & (col < (row + 1) * _DH)


def _softmax2(s):
    m = jnp.max(s, axis=-1, keepdims=True)
    p = jnp.exp2(s - m)
    return p * (1.0 / jnp.sum(p, axis=-1, keepdims=True))


def _tree_sum(ts):
    while len(ts) > 1:
        ts = [ts[i] + ts[i + 1] for i in range(0, len(ts), 2)]
    return ts[0]


def _col_bcast(row):
    return jnp.broadcast_to(row, (128, 128)).T


def _rows_total(c):
    return jnp.broadcast_to(jnp.sum(c, axis=0, keepdims=True), (8, 128))


def _q_blockdiag(xb, qs, wq_s, h0, gs):
    j0 = h0 * _DH // 128
    q = jnp.concatenate([_mm(xb, _ld(wq_s[j0 + c])) for c in range(gs * _DH // 128)], axis=1)
    return jnp.where(_head_mask(gs), q * qs, 0.0).astype(_BF)


def _probs(qbd, kb, h0, gs):
    rows = slice(h0 * _DH // 2, (h0 + gs) * _DH // 2)
    return _softmax2(jnp.concatenate([_mm(qbd, _ld(kb[j, rows, :])) for j in range(_NJ)], axis=1))


def _attn_resident(x, kb, vf, wq_s, wo_f):
    xc, rstd = _ln_parts(x)
    xb = xc.astype(_BF)
    qs = rstd * _QSCALE
    ng = _H // _GS
    q, p = {}, {}
    yacc = [jnp.zeros((8, 128), _F32)] * _ND

    def pv(g):
        for i in range(_GS):
            h = g * _GS + i
            pb = [jnp.broadcast_to(p[g][i:i + 1, 128 * j:128 * (j + 1)], (8, 128)) for j in range(_NJ)]
            for r in range(_DH // 8):
                r0 = h * _DH + 8 * r
                o = jnp.sum(_tree_sum([vf[j, r0:r0 + 8, :] * pb[j] for j in range(_NJ)]),
                            axis=-1, keepdims=True)
                for n in range(_ND):
                    yacc[n] = yacc[n] + wo_f[r0:r0 + 8, 128 * n:128 * (n + 1)] * o

    q[0] = _q_blockdiag(xb, qs, wq_s, 0, _GS)
    for g in range(ng + _LAG):
        if g + 1 < ng:
            q[g + 1] = _q_blockdiag(xb, qs, wq_s, (g + 1) * _GS, _GS)
        if g < ng:
            p[g] = _probs(q[g], kb, g * _GS, _GS)
        if g - _LAG >= 0:
            pv(g - _LAG)
    return x + jnp.concatenate([jnp.sum(y, axis=0, keepdims=True) for y in yacc], axis=1)


def _ffn(x, wr, wg_s, wu_s, wd_s, wgu_f, wd_f):
    xc, rstd = _ln_parts(x)
    xb = xc.astype(_BF)
    xr = xb.astype(_F32)
    r = jnp.sum(xr * wr, axis=-1, keepdims=True) * rstd
    nf = _F // 128
    nm = nf - _NV
    gate = [None] * nf
    up = [None] * nf
    for j in range(nm):
        gate[j] = _mm(xb, _ld(wg_s[j]))
        up[j] = _mm(xb, _ld(wu_s[j]))
    xcol = jnp.concatenate([_col_bcast(xr[0:1, 128 * i:128 * (i + 1)]) for i in range(_ND)], axis=0)
    acc = [None] * (2 * _NV)
    for kc in range(_D // 16):
        x2 = xcol[16 * kc:16 * kc + 16]
        for i in range(2 * _NV):
            t = wgu_f[i, 16 * kc:16 * kc + 16, :] * x2
            t = t[0:8] + t[8:16]
            acc[i] = t if acc[i] is None else acc[i] + t
    for i in range(_NV):
        gate[nm + i] = _rows_total(acc[i])
        up[nm + i] = _rows_total(acc[_NV + i])
    hs = []
    for j in range(nf):
        g = gate[j] * rstd
        hs.append((g * jax.nn.sigmoid(g) * (up[j] * rstd)).astype(_BF))
    hm = jnp.concatenate(hs[_KD:], axis=1)
    y = jnp.concatenate([_mm(hm, _ld(wd_s[64 * _KD:, 128 * n:128 * (n + 1)])) for n in range(_ND)], axis=1)
    ya = [None] * _ND
    for blk in range(_KD):
        hcol = _col_bcast(hs[blk].astype(_F32)[0:1, :])
        for rr in range(16):
            r0 = 128 * blk + 8 * rr
            for n in range(_ND):
                t = wd_f[r0:r0 + 8, 128 * n:128 * (n + 1)] * hcol[8 * rr:8 * rr + 8]
                ya[n] = t if ya[n] is None else ya[n] + t
    y = y + jnp.concatenate([_rows_total(c) for c in ya], axis=1)
    return x + (xc * rstd + y * jax.nn.sigmoid(r))


def _kernel(x_hbm, wr_hbm, k_hbm, v_hbm, wq_hbm, wo_hbm, wg_hbm, wu_hbm, wd_hbm, o_ref,
            kbuf, vbuf, wq_s, wo_s, wg_s, wu_s, wd_s, vf, wo_f, wgu_f, wd_f,
            x_s, wr_s, xs, ys, ps, ksem, vsem, wsem):
    def lanes(j):
        return pl.ds(pl.multiple_of(_SK - _W + 128 * j, 128), 128)

    def k_copy(b, j):
        return pltpu.make_async_copy(k_hbm.at[b, :, lanes(j)], kbuf.bitcast(_BF).at[b % 2, j], ksem.at[b % 2])

    def v_copy(b, c, j):
        h0, n = _V_CHUNKS[c]
        rows = pl.ds(h0 * _DH, n * _DH)
        return pltpu.make_async_copy(v_hbm.at[b, rows, lanes(j)], vbuf.bitcast(_BF).at[b % 2, j, rows],
                                     vsem.at[b % 2, c])

    def w_copy(src, dst, sem, j):
        return pltpu.make_async_copy(src.at[:, pl.ds(pl.multiple_of(128 * j, 128), 128)],
                                     dst.bitcast(_BF).at[j], wsem.at[sem])

    wq_c = functools.partial(w_copy, wq_hbm, wq_s, 0)
    wg_c = functools.partial(w_copy, wg_hbm, wg_s, 2)
    wu_c = functools.partial(w_copy, wu_hbm, wu_s, 3)
    wo_c = pltpu.make_async_copy(wo_hbm, wo_s.bitcast(_BF), wsem.at[1])
    wd_c = pltpu.make_async_copy(wd_hbm, wd_s.bitcast(_BF), wsem.at[4])
    x_c = pltpu.make_async_copy(x_hbm, x_s, wsem.at[5])
    wr_c = pltpu.make_async_copy(wr_hbm, wr_s, wsem.at[6])

    def start_all(n, copy):
        def body(j, carry):
            copy(j).start()
            return carry
        lax.fori_loop(0, n, body, 0)

    def wait_all(n, copy):
        for j in range(n):
            copy(j).wait()

    start_all(wq_s.shape[0], wq_c)
    x_c.start()
    wr_c.start()
    wo_c.start()
    start_all(wg_s.shape[0], wg_c)
    start_all(wu_s.shape[0], wu_c)
    wd_c.start()
    start_all(_NJ, lambda j: k_copy(0, j))
    for c in range(len(_V_CHUNKS)):
        start_all(_NJ, lambda j, c=c: v_copy(0, c, j))

    x_c.wait()
    wr_c.wait()
    xs[...] = jnp.zeros(xs.shape, _F32)
    xs[0:_B, :] = x_s[...].astype(_F32)
    ys[...] = jnp.zeros(ys.shape, _F32)
    wr = wr_s[...].astype(_F32).reshape(1, _D)

    wo_c.wait()

    def widen_wo(h, carry):
        wo_f[pl.ds(pl.multiple_of(h * _DH, 8), _DH), :] = _ld(
            wo_s[pl.ds(pl.multiple_of(h * (_DH // 2), 8), _DH // 2), :]).astype(_F32)
        return carry
    lax.fori_loop(0, _H, widen_wo, 0)

    wait_all(wq_s.shape[0], wq_c)
    wait_all(wg_s.shape[0], wg_c)
    wait_all(wu_s.shape[0], wu_c)
    wd_c.wait()
    for i in range(_NV):
        wgu_f[i] = _ld(wg_s[_F // 128 - _NV + i]).astype(_F32)
        wgu_f[_NV + i] = _ld(wu_s[_F // 128 - _NV + i]).astype(_F32)
    for blk in range(_KD):
        wd_f[128 * blk:128 * (blk + 1), :] = _ld(wd_s[64 * blk:64 * (blk + 1), :]).astype(_F32)

    def batch_body(b, carry):
        kb = kbuf.at[b % 2]
        vb = vbuf.at[b % 2]
        x = jnp.broadcast_to(xs[pl.ds(b, 1), :], (8, _D))

        @pl.when(b + 1 < _B)
        def _():
            start_all(_NJ, lambda j: k_copy(b + 1, j))
        wait_all(_NJ, lambda j: k_copy(b, j))

        xc, rstd = _ln_parts(x)
        xb = xc.astype(_BF)
        qs = rstd * _QSCALE
        for g in range(_H // 8):
            ps[8 * g:8 * g + 8, :] = _probs(_q_blockdiag(xb, qs, wq_s, 8 * g, 8), kb, 8 * g, 8)

        def head(h, ya):
            prow = ps[pl.ds(h, 1), :]
            pb = [jnp.broadcast_to(prow[:, 128 * j:128 * (j + 1)], (8, 128)) for j in range(_NJ)]
            ya = list(ya)
            for r in range(_DH // 16):
                r0 = pl.multiple_of(h * _DH + 16 * r, 8)
                w0 = pl.multiple_of(h * (_DH // 2) + 8 * r, 8)
                lo, hi = [], []
                for j in range(_NJ):
                    v = _ld(vb[j, pl.ds(w0, 8), :]).astype(_F32)
                    vf[j, pl.ds(r0, 16), :] = v
                    lo.append(v[0:8] * pb[j])
                    hi.append(v[8:16] * pb[j])
                for u, ts in enumerate((lo, hi)):
                    o = jnp.sum(_tree_sum(ts), axis=-1, keepdims=True)
                    for n in range(_ND):
                        ya[n] = ya[n] + wo_f[pl.ds(r0 + 8 * u, 8), 128 * n:128 * (n + 1)] * o
            return tuple(ya)

        ya = tuple(jnp.zeros((8, 128), _F32) for _ in range(_ND))
        for c, (h0, n) in enumerate(_V_CHUNKS):
            wait_all(_NJ, lambda j, c=c: v_copy(b, c, j))

            @pl.when(b + 1 < _B)
            def _(c=c):
                start_all(_NJ, lambda j: v_copy(b + 1, c, j))

            def pair(i, ya, h0=h0):
                return head(h0 + 2 * i + 1, head(h0 + 2 * i, ya))

            if n == 1:
                ya = head(h0, ya)
            elif n == 2:
                ya = pair(0, ya)
            else:
                ya = lax.fori_loop(0, n // 2, pair, ya)

        x = x + jnp.concatenate([jnp.sum(y, axis=0, keepdims=True) for y in ya], axis=1)
        x = _ffn(x, wr, wg_s, wu_s, wd_s, wgu_f, wd_f)
        x = _attn_resident(x, kb, vf, wq_s, wo_f)
        x = _ffn(x, wr, wg_s, wu_s, wd_s, wgu_f, wd_f)
        ys[pl.ds(b, 1), :] = x[0:1, :]
        return carry

    lax.fori_loop(0, _B, batch_body, 0)
    o_ref[...] = ys[0:_B, :].astype(o_ref.dtype)


@jax.jit
def pallas_interleave_layers__sliding_block_cached__moe_arch_mod__decode_kernel(
    A_x: jax.Array,
    A_k_cache: jax.Array,
    A_v_cache: jax.Array,
    A_wq: jax.Array,
    A_wo: jax.Array,
    B_x: jax.Array,
    B_w_r: jax.Array,
    B_w_gate: jax.Array,
    B_w_up: jax.Array,
    B_w_down: jax.Array,
):
    del B_x
    kt = jnp.transpose(A_k_cache, (0, 1, 3, 2)).reshape(_B, _H * _DH, _SK)
    vt = jnp.transpose(A_v_cache, (0, 1, 3, 2)).reshape(_B, _H * _DH, _SK)
    any_spec = pl.BlockSpec(memory_space=pl.ANY)
    out = pl.pallas_call(
        _kernel,
        out_shape=jax.ShapeDtypeStruct((_B, _D), A_x.dtype),
        in_specs=[any_spec] * 9,
        out_specs=pl.BlockSpec(memory_space=pltpu.VMEM),
        scratch_shapes=[
            pltpu.VMEM((2, _NJ, _H * _DH // 2, 128), _U32),
            pltpu.VMEM((2, _NJ, _H * _DH // 2, 128), _U32),
            pltpu.VMEM((_H * _DH // 128, _D // 2, 128), _U32),
            pltpu.VMEM((_H * _DH // 2, _D), _U32),
            pltpu.VMEM((_F // 128, _D // 2, 128), _U32),
            pltpu.VMEM((_F // 128, _D // 2, 128), _U32),
            pltpu.VMEM((_F // 2, _D), _U32),
            pltpu.VMEM((_NJ, _H * _DH, 128), _F32),
            pltpu.VMEM((_H * _DH, _D), _F32),
            pltpu.VMEM((2 * _NV, _D, 128), _F32),
            pltpu.VMEM((128 * _KD, _D), _F32),
            pltpu.VMEM((_B, _D), _BF),
            pltpu.VMEM((_D,), _BF),
            pltpu.VMEM((8, _D), _F32),
            pltpu.VMEM((8, _D), _F32),
            pltpu.VMEM((_H, _W), _F32),
            pltpu.SemaphoreType.DMA((2,)),
            pltpu.SemaphoreType.DMA((2, len(_V_CHUNKS))),
            pltpu.SemaphoreType.DMA((7,)),
        ],
        compiler_params=pltpu.CompilerParams(vmem_limit_bytes=116 * 1024 * 1024),
    )(A_x.reshape(_B, _D), B_w_r, kt, vt, A_wq, A_wo, B_w_gate, B_w_up, B_w_down)
    return out.reshape(_B, 1, _D)
```

```python
import functools

import jax
import jax.numpy as jnp
import numpy as np
from jax import lax
import jax.experimental.pallas as pl
import jax.experimental.pallas.tpu as pltpu

_D = 640
_H = 32
_DH = 192
_SK = 4096
_W = 1024
_F = 1536
_B = 4
_NJ = _W // 128
_ND = _D // 128
_EPS = 1e-5
_BF = jnp.bfloat16
_F32 = jnp.float32
_U32 = jnp.uint32

_V_CHUNKS = ((0, 8), (8, 8), (16, 8), (24, 4), (28, 2), (30, 1), (31, 1))
_GS = 2
_LAG = 4
_QV = (2, 3)
_NV = 2
_KD = 8
_QSCALE = float(_DH ** -0.5 * np.log2(np.e))


def _mm(a, b):
    return jnp.dot(a, b, preferred_element_type=_F32)


def _ld(words):
    return pltpu.bitcast(words, _BF)


def _ln_parts(x):
    xc = x - jnp.mean(x, axis=-1, keepdims=True)
    var = jnp.mean(xc * xc, axis=-1, keepdims=True)
    return xc, lax.rsqrt(var + _EPS)


def _head_mask(gs):
    row = lax.broadcasted_iota(jnp.int32, (8, gs * _DH), 0)
    col = lax.broadcasted_iota(jnp.int32, (8, gs * _DH), 1)
    return (col >= row * _DH) & (col < (row + 1) * _DH)


def _softmax2(s):
    m = jnp.max(s, axis=-1, keepdims=True)
    p = jnp.exp2(s - m)
    return p * (1.0 / jnp.sum(p, axis=-1, keepdims=True))


def _tree_sum(ts):
    while len(ts) > 1:
        ts = [ts[i] + ts[i + 1] for i in range(0, len(ts), 2)]
    return ts[0]


def _col_bcast(row):
    return jnp.broadcast_to(row, (128, 128)).T


def _rows_total(c):
    return jnp.broadcast_to(jnp.sum(c, axis=0, keepdims=True), (8, 128))


def _q_blockdiag(xb, qs, wq_s, h0, gs):
    j0 = h0 * _DH // 128
    q = jnp.concatenate([_mm(xb, _ld(wq_s[j0 + c])) for c in range(gs * _DH // 128)], axis=1)
    return jnp.where(_head_mask(gs), q * qs, 0.0).astype(_BF)


def _probs(qbd, kb, h0, gs):
    rows = slice(h0 * _DH // 2, (h0 + gs) * _DH // 2)
    return _softmax2(jnp.concatenate([_mm(qbd, _ld(kb[j, rows, :])) for j in range(_NJ)], axis=1))


def _attn_resident(x, kb, vf, wq_s, wo_f, wq_f):
    xc, rstd = _ln_parts(x)
    xb = xc.astype(_BF)
    qs = rstd * _QSCALE
    ng = _H // _GS
    q, p = {}, {}
    yacc = [jnp.zeros((8, 128), _F32)] * _ND

    def pv(g):
        for i in range(_GS):
            h = g * _GS + i
            pb = [jnp.broadcast_to(p[g][i:i + 1, 128 * j:128 * (j + 1)], (8, 128)) for j in range(_NJ)]
            for r in range(_DH // 8):
                r0 = h * _DH + 8 * r
                o = jnp.sum(_tree_sum([vf[j, r0:r0 + 8, :] * pb[j] for j in range(_NJ)]),
                            axis=-1, keepdims=True)
                for n in range(_ND):
                    yacc[n] = yacc[n] + wo_f[r0:r0 + 8, 128 * n:128 * (n + 1)] * o

    q[0] = _q_blockdiag(xb, qs, wq_s, 0, _GS)
    xr = xb.astype(_F32)
    xcol = jnp.concatenate([_col_bcast(xr[0:1, 128 * i:128 * (i + 1)]) for i in range(_ND)], axis=0)
    nc = _GS * _DH // 128
    acc = [None] * (nc * len(_QV))
    for kc in range(_D // 16):
        x2 = xcol[16 * kc:16 * kc + 16]
        for i in range(len(acc)):
            t = wq_f[i, 16 * kc:16 * kc + 16, :] * x2
            t = t[0:8] + t[8:16]
            acc[i] = t if acc[i] is None else acc[i] + t
    for i, g in enumerate(_QV):
        qv = jnp.concatenate([_rows_total(acc[i * nc + c]) for c in range(nc)], axis=1)
        q[g] = jnp.where(_head_mask(_GS), qv * qs, 0.0).astype(_BF)
    for g in range(ng + _LAG):
        if g + 1 < ng and g + 1 not in _QV:
            q[g + 1] = _q_blockdiag(xb, qs, wq_s, (g + 1) * _GS, _GS)
        if g < ng:
            p[g] = _probs(q[g], kb, g * _GS, _GS)
        if g - _LAG >= 0:
            pv(g - _LAG)
    return x + jnp.concatenate([jnp.sum(y, axis=0, keepdims=True) for y in yacc], axis=1)


def _ffn(x, wr, wg_s, wu_s, wd_s, wgu_f, wd_f):
    xc, rstd = _ln_parts(x)
    xb = xc.astype(_BF)
    xr = xb.astype(_F32)
    r = jnp.sum(xr * wr, axis=-1, keepdims=True) * rstd
    nf = _F // 128
    nm = nf - _NV
    gate = [None] * nf
    up = [None] * nf
    for j in range(nm):
        gate[j] = _mm(xb, _ld(wg_s[j]))
        up[j] = _mm(xb, _ld(wu_s[j]))
    xcol = jnp.concatenate([_col_bcast(xr[0:1, 128 * i:128 * (i + 1)]) for i in range(_ND)], axis=0)
    acc = [None] * (2 * _NV)
    for kc in range(_D // 16):
        x2 = xcol[16 * kc:16 * kc + 16]
        for i in range(2 * _NV):
            t = wgu_f[i, 16 * kc:16 * kc + 16, :] * x2
            t = t[0:8] + t[8:16]
            acc[i] = t if acc[i] is None else acc[i] + t
    for i in range(_NV):
        gate[nm + i] = _rows_total(acc[i])
        up[nm + i] = _rows_total(acc[_NV + i])
    hs = []
    for j in range(nf):
        g = gate[j] * rstd
        hs.append((g * jax.nn.sigmoid(g) * (up[j] * rstd)).astype(_BF))
    hm = jnp.concatenate(hs[_KD:], axis=1)
    y = jnp.concatenate([_mm(hm, _ld(wd_s[64 * _KD:, 128 * n:128 * (n + 1)])) for n in range(_ND)], axis=1)
    ya = [None] * _ND
    for blk in range(_KD):
        hcol = _col_bcast(hs[blk].astype(_F32)[0:1, :])
        for rr in range(16):
            r0 = 128 * blk + 8 * rr
            for n in range(_ND):
                t = wd_f[r0:r0 + 8, 128 * n:128 * (n + 1)] * hcol[8 * rr:8 * rr + 8]
                ya[n] = t if ya[n] is None else ya[n] + t
    y = y + jnp.concatenate([_rows_total(c) for c in ya], axis=1)
    return x + (xc * rstd + y * jax.nn.sigmoid(r))


def _kernel(x_hbm, wr_hbm, k_hbm, v_hbm, wq_hbm, wo_hbm, wg_hbm, wu_hbm, wd_hbm, o_ref,
            kbuf, vbuf, wq_s, wo_s, wg_s, wu_s, wd_s, vf, wo_f, wgu_f, wd_f, wq_f,
            x_s, wr_s, xs, ys, ps, ksem, vsem, wsem):
    def lanes(j):
        return pl.ds(pl.multiple_of(_SK - _W + 128 * j, 128), 128)

    def k_copy(b, j):
        return pltpu.make_async_copy(k_hbm.at[b, :, lanes(j)], kbuf.bitcast(_BF).at[b % 2, j], ksem.at[b % 2])

    def v_copy(b, c, j):
        h0, n = _V_CHUNKS[c]
        rows = pl.ds(h0 * _DH, n * _DH)
        return pltpu.make_async_copy(v_hbm.at[b, rows, lanes(j)], vbuf.bitcast(_BF).at[b % 2, j, rows],
                                     vsem.at[b % 2, c])

    def w_copy(src, dst, sem, j):
        return pltpu.make_async_copy(src.at[:, pl.ds(pl.multiple_of(128 * j, 128), 128)],
                                     dst.bitcast(_BF).at[j], wsem.at[sem])

    wq_c = functools.partial(w_copy, wq_hbm, wq_s, 0)
    wg_c = functools.partial(w_copy, wg_hbm, wg_s, 2)
    wu_c = functools.partial(w_copy, wu_hbm, wu_s, 3)
    wo_c = pltpu.make_async_copy(wo_hbm, wo_s.bitcast(_BF), wsem.at[1])
    wd_c = pltpu.make_async_copy(wd_hbm, wd_s.bitcast(_BF), wsem.at[4])
    x_c = pltpu.make_async_copy(x_hbm, x_s, wsem.at[5])
    wr_c = pltpu.make_async_copy(wr_hbm, wr_s, wsem.at[6])

    def start_all(n, copy):
        def body(j, carry):
            copy(j).start()
            return carry
        lax.fori_loop(0, n, body, 0)

    def wait_all(n, copy):
        for j in range(n):
            copy(j).wait()

    start_all(wq_s.shape[0], wq_c)
    x_c.start()
    wr_c.start()
    wo_c.start()
    start_all(wg_s.shape[0], wg_c)
    start_all(wu_s.shape[0], wu_c)
    wd_c.start()
    start_all(_NJ, lambda j: k_copy(0, j))
    for c in range(len(_V_CHUNKS)):
        start_all(_NJ, lambda j, c=c: v_copy(0, c, j))

    x_c.wait()
    wr_c.wait()
    xs[...] = jnp.zeros(xs.shape, _F32)
    xs[0:_B, :] = x_s[...].astype(_F32)
    ys[...] = jnp.zeros(ys.shape, _F32)
    wr = wr_s[...].astype(_F32).reshape(1, _D)

    wo_c.wait()

    def widen_wo(h, carry):
        wo_f[pl.ds(pl.multiple_of(h * _DH, 8), _DH), :] = _ld(
            wo_s[pl.ds(pl.multiple_of(h * (_DH // 2), 8), _DH // 2), :]).astype(_F32)
        return carry
    lax.fori_loop(0, _H, widen_wo, 0)

    wait_all(wq_s.shape[0], wq_c)
    wait_all(wg_s.shape[0], wg_c)
    wait_all(wu_s.shape[0], wu_c)
    wd_c.wait()
    for i in range(_NV):
        wgu_f[i] = _ld(wg_s[_F // 128 - _NV + i]).astype(_F32)
        wgu_f[_NV + i] = _ld(wu_s[_F // 128 - _NV + i]).astype(_F32)
    for i, g in enumerate(_QV):
        for c in range(_GS * _DH // 128):
            wq_f[i * (_GS * _DH // 128) + c] = _ld(wq_s[g * (_GS * _DH // 128) + c]).astype(_F32)
    for blk in range(_KD):
        wd_f[128 * blk:128 * (blk + 1), :] = _ld(wd_s[64 * blk:64 * (blk + 1), :]).astype(_F32)

    def batch_body(b, carry):
        kb = kbuf.at[b % 2]
        vb = vbuf.at[b % 2]
        x = jnp.broadcast_to(xs[pl.ds(b, 1), :], (8, _D))

        @pl.when(b + 1 < _B)
        def _():
            start_all(_NJ, lambda j: k_copy(b + 1, j))
        wait_all(_NJ, lambda j: k_copy(b, j))

        xc, rstd = _ln_parts(x)
        xb = xc.astype(_BF)
        qs = rstd * _QSCALE
        for g in range(_H // 8):
            ps[8 * g:8 * g + 8, :] = _probs(_q_blockdiag(xb, qs, wq_s, 8 * g, 8), kb, 8 * g, 8)

        def head(h, ya):
            prow = ps[pl.ds(h, 1), :]
            pb = [jnp.broadcast_to(prow[:, 128 * j:128 * (j + 1)], (8, 128)) for j in range(_NJ)]
            ya = list(ya)
            for r in range(_DH // 16):
                r0 = pl.multiple_of(h * _DH + 16 * r, 8)
                w0 = pl.multiple_of(h * (_DH // 2) + 8 * r, 8)
                lo, hi = [], []
                for j in range(_NJ):
                    v = _ld(vb[j, pl.ds(w0, 8), :]).astype(_F32)
                    vf[j, pl.ds(r0, 16), :] = v
                    lo.append(v[0:8] * pb[j])
                    hi.append(v[8:16] * pb[j])
                for u, ts in enumerate((lo, hi)):
                    o = jnp.sum(_tree_sum(ts), axis=-1, keepdims=True)
                    for n in range(_ND):
                        ya[n] = ya[n] + wo_f[pl.ds(r0 + 8 * u, 8), 128 * n:128 * (n + 1)] * o
            return tuple(ya)

        ya = tuple(jnp.zeros((8, 128), _F32) for _ in range(_ND))
        for c, (h0, n) in enumerate(_V_CHUNKS):
            wait_all(_NJ, lambda j, c=c: v_copy(b, c, j))

            @pl.when(b + 1 < _B)
            def _(c=c):
                start_all(_NJ, lambda j: v_copy(b + 1, c, j))

            def pair(i, ya, h0=h0):
                return head(h0 + 2 * i + 1, head(h0 + 2 * i, ya))

            if n == 1:
                ya = head(h0, ya)
            elif n == 2:
                ya = pair(0, ya)
            else:
                ya = lax.fori_loop(0, n // 2, pair, ya)

        x = x + jnp.concatenate([jnp.sum(y, axis=0, keepdims=True) for y in ya], axis=1)
        x = _ffn(x, wr, wg_s, wu_s, wd_s, wgu_f, wd_f)
        x = _attn_resident(x, kb, vf, wq_s, wo_f, wq_f)
        x = _ffn(x, wr, wg_s, wu_s, wd_s, wgu_f, wd_f)
        ys[pl.ds(b, 1), :] = x[0:1, :]
        return carry

    lax.fori_loop(0, _B, batch_body, 0)
    o_ref[...] = ys[0:_B, :].astype(o_ref.dtype)


@jax.jit
def pallas_interleave_layers__sliding_block_cached__moe_arch_mod__decode_kernel(
    A_x: jax.Array,
    A_k_cache: jax.Array,
    A_v_cache: jax.Array,
    A_wq: jax.Array,
    A_wo: jax.Array,
    B_x: jax.Array,
    B_w_r: jax.Array,
    B_w_gate: jax.Array,
    B_w_up: jax.Array,
    B_w_down: jax.Array,
):
    del B_x
    kt = jnp.transpose(A_k_cache, (0, 1, 3, 2)).reshape(_B, _H * _DH, _SK)
    vt = jnp.transpose(A_v_cache, (0, 1, 3, 2)).reshape(_B, _H * _DH, _SK)
    any_spec = pl.BlockSpec(memory_space=pl.ANY)
    out = pl.pallas_call(
        _kernel,
        out_shape=jax.ShapeDtypeStruct((_B, _D), A_x.dtype),
        in_specs=[any_spec] * 9,
        out_specs=pl.BlockSpec(memory_space=pltpu.VMEM),
        scratch_shapes=[
            pltpu.VMEM((2, _NJ, _H * _DH // 2, 128), _U32),
            pltpu.VMEM((2, _NJ, _H * _DH // 2, 128), _U32),
            pltpu.VMEM((_H * _DH // 128, _D // 2, 128), _U32),
            pltpu.VMEM((_H * _DH // 2, _D), _U32),
            pltpu.VMEM((_F // 128, _D // 2, 128), _U32),
            pltpu.VMEM((_F // 128, _D // 2, 128), _U32),
            pltpu.VMEM((_F // 2, _D), _U32),
            pltpu.VMEM((_NJ, _H * _DH, 128), _F32),
            pltpu.VMEM((_H * _DH, _D), _F32),
            pltpu.VMEM((2 * _NV, _D, 128), _F32),
            pltpu.VMEM((128 * _KD, _D), _F32),
            pltpu.VMEM((len(_QV) * _GS * _DH // 128, _D, 128), _F32),
            pltpu.VMEM((_B, _D), _BF),
            pltpu.VMEM((_D,), _BF),
            pltpu.VMEM((8, _D), _F32),
            pltpu.VMEM((8, _D), _F32),
            pltpu.VMEM((_H, _W), _F32),
            pltpu.SemaphoreType.DMA((2,)),
            pltpu.SemaphoreType.DMA((2, len(_V_CHUNKS))),
            pltpu.SemaphoreType.DMA((7,)),
        ],
        compiler_params=pltpu.CompilerParams(vmem_limit_bytes=116 * 1024 * 1024),
    )(A_x.reshape(_B, _D), B_w_r, kt, vt, A_wq, A_wo, B_w_gate, B_w_up, B_w_down)
    return out.reshape(_B, 1, _D)
```
